```python
import jax
import jax.numpy as jnp

def _softmax(x, axis=-1):
    return jax.nn.softmax(x, axis=axis)

def _gelu(x):
    return jax.nn.gelu(x, approximate=True)

def _silu(x):
    return jax.nn.silu(x)

def _sigmoid(x):
    return jax.nn.sigmoid(x)

def _layernorm(x, axis=-1, eps=1e-05):
    m = jnp.mean(x, axis=axis, keepdims=True)
    v = jnp.var(x, axis=axis, keepdims=True)
    return (x - m) / jnp.sqrt(v + eps)

def _scatter_add(tgt, idx, src, axis=0):
    return tgt.at[idx].add(src)

def _segment_sum(src, seg, n):
    return jax.ops.segment_sum(src, seg, n)

class _Rng:

    def __init__(self, key):
        self._k = key

    def _next(self):
        self._k, sub = jax.random.split(self._k)
        return sub

    def normal(self, shape):
        return jax.random.normal(self._next(), shape, dtype=jnp.bfloat16)

    def randint(self, lo, hi, shape):
        return jax.random.randint(self._next(), shape, lo, hi, dtype=jnp.int32)

    def uniform(self, shape, lo=0.0, hi=1.0):
        return jax.random.uniform(self._next(), shape, jnp.bfloat16, lo, hi)

    def permutation(self, n):
        return jax.random.permutation(self._next(), n)
kernel_name = 'interleave_layers__memory_aug_infini_attn__sliding_local_dilated__prompt'

def setup_inputs():
    _rng = _Rng(jax.random.key(int.from_bytes(__import__("os").urandom(4), "little")))
    _w = lambda a: (lambda t: t.astype(jnp.bfloat16) if jnp.issubdtype(t.dtype, jnp.floating) else t)(jnp.asarray(a))

    def _A_setup():
        B, S, D, H = (1, 2048, 1024, 32)
        N = 4
        L = max(1, S // N)
        sc = D ** (-0.5)
        return {'x': _w((lambda *s: _rng.normal(s) * 0.05)(B, N * L, D)), 'wq': _w((lambda *s: _rng.normal(s) * 0.05)(D, D) * sc), 'wk': _w((lambda *s: _rng.normal(s) * 0.05)(D, D) * sc), 'wv': _w((lambda *s: _rng.normal(s) * 0.05)(D, D) * sc), 'wo': _w((lambda *s: _rng.normal(s) * 0.05)(D, D) * sc), 'beta': _w((lambda *s: _rng.normal(s) * 0.05)(H))}
    _A_in = _A_setup()

    def _B_setup():
        B, S, D = (1, 2048, 1024)
        return {'x': _w((lambda *s: _rng.normal(s) * 0.05)(B, S, D)), 'wqkv': _w((lambda *s: _rng.normal(s) * 0.05)(D, 3 * D)), 'wo': _w((lambda *s: _rng.normal(s) * 0.05)(D, D))}
    _B_in = _B_setup()
    return {'A_x': _A_in['x'], 'A_wq': _A_in['wq'], 'A_wk': _A_in['wk'], 'A_wv': _A_in['wv'], 'A_wo': _A_in['wo'], 'A_beta': _A_in['beta'], 'B_x': _B_in['x'], 'B_wqkv': _B_in['wqkv'], 'B_wo': _B_in['wo']}

def reference(A_x, A_wq, A_wk, A_wv, A_wo, A_beta, B_x, B_wqkv, B_wo):

    def _A_ref(x, wq, wk, wv, wo, beta):
        B, S, D = x.shape
        H = 32
        Dh = D // H
        N = 4
        L = S // N
        q = (lambda x, *d: x.transpose(*d))((x @ wq).reshape(B, S, H, Dh), 0, 2, 1, 3).reshape(B, H, N, L, Dh)
        k = (lambda x, *d: x.transpose(*d))((x @ wk).reshape(B, S, H, Dh), 0, 2, 1, 3).reshape(B, H, N, L, Dh)
        v = (lambda x, *d: x.transpose(*d))((x @ wv).reshape(B, S, H, Dh), 0, 2, 1, 3).reshape(B, H, N, L, Dh)
        phi = lambda t: jnp.where(t > 0, t + 1.0, jnp.exp(t))
        scale = Dh ** (-0.5)
        ar = jnp.arange(L)
        mask = (lambda x, dt: x.astype(dt))(ar[:, None] < ar[None, :], x.dtype) * -1000000000.0
        g = _sigmoid(beta).reshape(1, H, 1, 1)
        M = jnp.einsum('bhd,bhe->bhde', q[:, :, 0, 0, :] * 0.0, q[:, :, 0, 0, :] * 0.0)
        z = q[:, :, 0, 0, :] * 0.0
        outs = []
        for s in range(N):
            qs, ks, vs = (q[:, :, s].copy(), k[:, :, s].copy(), v[:, :, s].copy())
            logits = jnp.einsum('bhqd,bhkd->bhqk', qs, ks) * scale + mask
            p = _softmax(logits, axis=-1)
            a_dot = jnp.einsum('bhqk,bhkd->bhqd', p, vs)
            pq = phi(qs)
            num = jnp.einsum('bhld,bhde->bhle', pq, M)
            den = jnp.einsum('bhld,bhd->bhl', pq, z)[..., None] + 1e-06
            a_mem = num / den
            o = g * a_mem + (1.0 - g) * a_dot
            outs.append(o)
            pk = phi(ks)
            M = M + jnp.einsum('bhld,bhle->bhde', pk, vs)
            z = z + jnp.einsum('bhld->bhd', pk)
        o = (lambda x, *d: x.transpose(*d))(jnp.stack(outs, 2).reshape(B, H, S, Dh), 0, 2, 1, 3).reshape(B, S, D)
        return o @ wo

    def _B_ref(x, wqkv, wo):
        B, S, D = x.shape
        H = 32
        Dh = D // H
        W, dil = (8, 2)
        qkv = (lambda x, *d: x.transpose(*d))((x @ wqkv).reshape(B, S, 3, H, Dh), 2, 0, 3, 1, 4)
        q, k, v = (qkv[0], qkv[1], qkv[2])
        scale = Dh ** (-0.5)
        pos = jnp.arange(S)
        off = jnp.arange(W) * dil
        idx = pos[:, None] - off[None, :]
        mask = idx >= 0
        idx_c = jnp.where(mask, idx, 0).reshape(-1)
        kg = k[:, :, idx_c, :].reshape(B, H, S, W, Dh)
        vg = v[:, :, idx_c, :].reshape(B, H, S, W, Dh)
        logits = jnp.einsum('bhsd,bhswd->bhsw', q, kg) * scale
        logits = jnp.where(mask[None, None, :, :], logits, -1000000000.0)
        attn = _softmax(logits, axis=-1)
        o = jnp.einsum('bhsw,bhswd->bhsd', attn, vg)
        return (lambda x, *d: x.transpose(*d))(o, 0, 2, 1, 3).reshape(B, S, D) @ wo
    x = A_x
    x = x + _A_ref(_layernorm(x, axis=-1), A_wq, A_wk, A_wv, A_wo, A_beta)
    x = x + _B_ref(_layernorm(x, axis=-1), B_wqkv, B_wo)
    x = x + _A_ref(_layernorm(x, axis=-1), A_wq, A_wk, A_wv, A_wo, A_beta)
    x = x + _B_ref(_layernorm(x, axis=-1), B_wqkv, B_wo)
    return x
```

```python
import functools
import math

import jax
import jax.numpy as jnp
from jax import lax
import jax.experimental.pallas as pl
import jax.experimental.pallas.tpu as pltpu

F32 = jnp.float32
BF16 = jnp.bfloat16

S, D, H, DH = 2048, 1024, 32, 32
NSEG, L = 4, 512
NG = D // 128
W, DIL = 8, 2
HALO = 16
LOG2E = 1.4426950408889634
QSCALE = (DH ** -0.5) * LOG2E
NEG = -1e30
PST = 33

CFG = dict(RB=128)


def _nn(a, b):
    return jnp.dot(a, b, preferred_element_type=F32)


def _nt(a, b):
    return lax.dot_general(a, b, (((1,), (1,)), ((), ())), preferred_element_type=F32)


def _ln(x):
    m = jnp.mean(x, axis=-1, keepdims=True)
    xc = x - m
    v = jnp.mean(xc * xc, axis=-1, keepdims=True)
    return (xc * lax.rsqrt(v + 1e-5)).astype(BF16)


def _phi(t):
    return jnp.where(t > 0, t + 1.0, jnp.exp(t))


def _kernel(x_hbm, wq_hbm, wk_hbm, wv_hbm, wo_hbm, beta_ref, wqkv_hbm, wob_hbm, out_ref,
            xin, wq, wk, wv, wo, wqkv, wob, wvt, wpt, wobp, pbuf,
            xres, xna, xnb, obuf, gate, mt, zs, qb, kb, vb, sems):
    it = pl.program_id(0)
    seg = it % NSEG
    nseg = (it + 1) % NSEG
    RB = CFG["RB"]

    @pl.when(it == 0)
    def _prologue():
        srcs = (x_hbm, wv_hbm, wq_hbm, wk_hbm, wo_hbm, wqkv_hbm, wob_hbm)
        dsts = (xin, wv, wq, wk, wo, wqkv, wob)
        cps = [pltpu.make_async_copy(s, d, sems.at[i]) for i, (s, d) in enumerate(zip(srcs, dsts))]
        for c in cps:
            c.start()
        g = jax.nn.sigmoid(beta_ref[...].astype(F32).reshape(1, H))
        r = lax.broadcasted_iota(jnp.int32, (H, H), 0)
        c = lax.broadcasted_iota(jnp.int32, (H, H), 1)
        col = jnp.sum(jnp.where(r == c, jnp.broadcast_to(g, (H, H)), 0.0), axis=1, keepdims=True)
        gate[...] = jnp.broadcast_to(col, (H, 128))
        cps[0].wait()
        x0 = xin[0:L, :].astype(F32)
        xres[0] = x0
        xna[...] = _ln(x0)
        cps[1].wait()
        wvt[...] = wv[...].T
        cps[2].wait()
        cps[3].wait()
        cps[4].wait()
        cps[5].wait()

        def perm_cols(i, carry):
            part = i // NG
            kt = i % NG
            k0 = pl.multiple_of(kt * 128, 128)
            n0 = pl.multiple_of(part * D, D)
            t = wqkv[pl.ds(k0, 128), pl.ds(n0, D)].T.astype(F32)
            for h in range(H):
                pbuf[pl.ds(h, DH, stride=PST), :] = t[h * DH:(h + 1) * DH]
            for d in range(DH):
                wpt[pl.ds(n0 + d * H, H), pl.ds(k0, 128)] = pbuf[pl.ds(d * PST, H), :].astype(BF16)
            return carry

        lax.fori_loop(0, 3 * NG, perm_cols, 0)
        cps[6].wait()

        def perm_rows(nt, carry):
            n0 = pl.multiple_of(nt * 128, 128)
            t = wob[:, pl.ds(n0, 128)].astype(F32)
            for h in range(H):
                pbuf[pl.ds(h, DH, stride=PST), :] = t[h * DH:(h + 1) * DH]
            for d in range(DH):
                wobp[pl.ds(d * H, H), pl.ds(n0, 128)] = pbuf[pl.ds(d * PST, H), :].astype(BF16)
            return carry

        lax.fori_loop(0, NG, perm_rows, 0)

    @pl.when(seg == 0)
    def _reset():
        mt[...] = jnp.zeros(mt.shape, F32)
        zs[...] = jnp.zeros(zs.shape, F32)
        kb[:, L:L + HALO, :] = jnp.zeros((NG, HALO, 128), F32)
        vb[:, L:L + HALO, :] = jnp.zeros((NG, HALO, 128), F32)

    lane_head = lax.broadcasted_iota(jnp.int32, (128, 128), 1) // DH
    row_head = lax.broadcasted_iota(jnp.int32, (128, 128), 0) // DH
    causal = (lax.broadcasted_iota(jnp.int32, (128, 512), 0)
              <= lax.broadcasted_iota(jnp.int32, (128, 512), 1) % 128)
    zrow = lax.broadcasted_iota(jnp.int32, (16, 128), 0)
    zlane = lax.broadcasted_iota(jnp.int32, (16, 128), 1) // DH

    st = [dict() for _ in range(NG)]

    def proj_q(g):
        q = _nn(xna[...], wq[:, g * 128:(g + 1) * 128])
        st[g]["qs"] = (q * QSCALE).astype(BF16)
        st[g]["pq"] = _phi(q).astype(BF16)

    def proj_k(g):
        k = _nn(xna[...], wk[:, g * 128:(g + 1) * 128])
        st[g]["k"] = k.astype(BF16)
        pk = _phi(k)
        st[g]["pk"] = pk.astype(BF16)
        st[g]["pksum"] = jnp.sum(pk, axis=0, keepdims=True)

    def proj_v(g):
        st[g]["vt"] = _nt(wvt[g * 128:(g + 1) * 128, :], xna[...]).astype(BF16)

    def qk(g, j):
        qj = st[g]["qs"][j * 128:(j + 1) * 128]
        qm = jnp.concatenate([jnp.where(lane_head == h, qj, jnp.zeros_like(qj)) for h in range(4)], axis=0)
        s = _nt(st[g]["k"][0:(j + 1) * 128], qm)
        sd = jnp.where(causal, s[j * 128:], NEG)
        s = jnp.concatenate([s[:j * 128], sd], axis=0) if j else sd
        m = jnp.max(s, axis=0, keepdims=True)
        p = jnp.exp2(s - m)
        st[g]["l", j] = jnp.sum(p, axis=0, keepdims=True)
        st[g]["p", j] = p.astype(BF16)

    def pv(g, j):
        outs = []
        for h in range(4):
            o = _nn(st[g]["vt"][h * DH:(h + 1) * DH, 0:(j + 1) * 128], st[g]["p", j][:, h * 128:(h + 1) * 128])
            gh = gate[4 * g + h:4 * g + h + 1, :]
            outs.append(o * ((1.0 - gh) / st[g]["l", j][:, h * 128:(h + 1) * 128]))
        st[g]["o", j] = jnp.concatenate(outs, axis=0)

    def mem(g):
        zm = jnp.where(zrow == zlane, jnp.broadcast_to(zs[g:g + 1, :], (16, 128)), 0.0)
        lhs = jnp.concatenate([mt[g], zm], axis=0).astype(BF16)
        r = _nt(lhs, st[g]["pq"])
        outs = []
        for h in range(4):
            gh = gate[4 * g + h:4 * g + h + 1, :]
            gh = jnp.concatenate([gh] * 4, axis=1)
            outs.append(r[h * DH:(h + 1) * DH] * (gh / (r[128 + h:128 + h + 1] + 1e-6)))
        st[g]["am"] = jnp.concatenate(outs, axis=0)

    def upd(g):
        u = _nn(st[g]["vt"], st[g]["pk"])
        mt[g] = mt[g] + jnp.where(lane_head == row_head, u, 0.0)
        zs[g:g + 1, :] = zs[g:g + 1, :] + st[g]["pksum"]

    def fin(g):
        ot = jnp.concatenate([st[g]["o", j] for j in range(4)], axis=1) + st[g]["am"]
        obuf[:, g * 128:(g + 1) * 128] = ot.astype(BF16).T

    proj_q(0); proj_k(0); proj_v(0)
    for g in range(NG):
        last = g == NG - 1
        qk(g, 3); qk(g, 2)
        if not last: proj_q(g + 1)
        pv(g, 3); pv(g, 2)
        qk(g, 1); qk(g, 0)
        mem(g); upd(g)
        if not last: proj_k(g + 1)
        pv(g, 1); pv(g, 0)
        if not last: proj_v(g + 1)
        fin(g)

    for i in range(L // RB):
        rows = slice(i * RB, (i + 1) * RB)
        x = xres[seg, rows, :] + _nn(obuf[rows, :], wo[...])
        xres[seg, rows, :] = x
        xnb[rows, :] = _ln(x)

    kb[:, 0:HALO, :] = kb[:, L:L + HALO, :]
    vb[:, 0:HALO, :] = vb[:, L:L + HALO, :]

    def b_proj(i):
        r0 = i * RB
        xn = xnb[r0:r0 + RB, :]
        for part, dst, off in ((0, qb, 0), (1, kb, HALO), (2, vb, HALO)):
            y = _nt(xn, wpt[part * D:(part + 1) * D, :])
            if part == 0:
                y = y * QSCALE
            for t in range(NG):
                dst[t, off + r0:off + r0 + RB, :] = y[:, t * 128:(t + 1) * 128]

    def b_attn(r0, R):
        acc = [None] * W
        for t in range(NG):
            q = qb[t, r0:r0 + R, :]
            for c in range(4):
                ks = kb[t, pl.ds(HALO + r0 - DIL * c - 8, R + 8), :]
                for w, kk in ((c, ks[8:]), (c + 4, ks[:R])):
                    acc[w] = q * kk if t == 0 else acc[w] + q * kk
        lg = []
        for w in range(W):
            a = acc[w]
            a = a + pltpu.roll(a, 64, 1)
            a = a + pltpu.roll(a, 32, 1)
            if r0 < DIL * w:
                pos = seg * L + r0 + lax.broadcasted_iota(jnp.int32, (R, 128), 0)
                a = jnp.where(pos >= DIL * w, a, NEG)
            lg.append(a)
        m = functools.reduce(jnp.maximum, lg)
        e = [jnp.exp2(a - m) for a in lg]
        inv = 1.0 / functools.reduce(lambda a, b: a + b, e)
        p = [a * inv for a in e]
        for t in range(NG):
            o = None
            for c in range(4):
                vs = vb[t, pl.ds(HALO + r0 - DIL * c - 8, R + 8), :]
                for w, vv in ((c, vs[8:]), (c + 4, vs[:R])):
                    o = p[w] * vv if o is None else o + p[w] * vv
            obuf[r0:r0 + R, t * 128:(t + 1) * 128] = o.astype(BF16)

    def b_out(i):
        rows = slice(i * RB, (i + 1) * RB)
        x = xres[seg, rows, :] + _nn(obuf[rows, :], wobp[...])
        xres[seg, rows, :] = x
        out_ref[rows, :] = x.astype(out_ref.dtype)

    def next_ln(i):
        rows = slice(i * RB, (i + 1) * RB)
        xi = xin[pl.ds(pl.multiple_of(nseg * L + i * RB, RB), RB), :].astype(F32)
        x = jnp.where(it < NSEG - 1, xi, xres[nseg, rows, :])
        xres[nseg, rows, :] = x
        xna[rows, :] = _ln(x)

    nb = L // RB
    for i in range(nb):
        b_proj(i)
        next_ln(i)
        if i > 0:
            for r in range((i - 1) * RB, i * RB, 32):
                b_attn(r, 32)
    for i in range(nb):
        b_out(i)
        if i == 0:
            for r in range((nb - 1) * RB, nb * RB, 32):
                b_attn(r, 32)


@jax.jit
def pallas_interleave_layers__memory_aug_infini_attn__sliding_local_dilated__prompt_kernel(A_x, A_wq, A_wk, A_wv, A_wo, A_beta, B_x, B_wqkv, B_wo):
    del B_x
    any_spec = pl.BlockSpec(memory_space=pl.ANY)
    out = pl.pallas_call(
        _kernel,
        grid=(2 * NSEG,),
        in_specs=[any_spec] * 5 + [pl.BlockSpec((H,), lambda i: (0,))] + [any_spec] * 2,
        out_specs=pl.BlockSpec((L, D), lambda i: (jnp.maximum(i - NSEG, 0), 0)),
        out_shape=jax.ShapeDtypeStruct((S, D), A_x.dtype),
        scratch_shapes=[
            pltpu.VMEM((S, D), BF16),
            pltpu.VMEM((D, D), BF16),
            pltpu.VMEM((D, D), BF16),
            pltpu.VMEM((D, D), BF16),
            pltpu.VMEM((D, D), BF16),
            pltpu.VMEM((D, 3 * D), BF16),
            pltpu.VMEM((D, D), BF16),
            pltpu.VMEM((D, D), BF16),
            pltpu.VMEM((3 * D, D), BF16),
            pltpu.VMEM((D, D), BF16),
            pltpu.VMEM((DH * PST, 128), F32),
            pltpu.VMEM((NSEG, L, D), F32),
            pltpu.VMEM((L, D), BF16),
            pltpu.VMEM((L, D), BF16),
            pltpu.VMEM((L, D), BF16),
            pltpu.VMEM((H, 128), F32),
            pltpu.VMEM((NG, 128, 128), F32),
            pltpu.VMEM((NG, 128), F32),
            pltpu.VMEM((NG, L, 128), F32),
            pltpu.VMEM((NG, L + HALO, 128), F32),
            pltpu.VMEM((NG, L + HALO, 128), F32),
            pltpu.SemaphoreType.DMA((8,)),
        ],
        compiler_params=pltpu.CompilerParams(
            dimension_semantics=("arbitrary",), vmem_limit_bytes=110 * 1024 * 1024),
        name="fused_layers",
    )(A_x.reshape(S, D), A_wq, A_wk, A_wv, A_wo, A_beta, B_wqkv, B_wo)
    return out.reshape(A_x.shape)
```

```python
import functools

import jax
import jax.numpy as jnp
from jax import lax
import jax.experimental.pallas as pl
import jax.experimental.pallas.tpu as pltpu

F32 = jnp.float32
BF16 = jnp.bfloat16
I32 = jnp.int32

S, D, H, DH = 2048, 1024, 32, 32
NSEG, L = 4, 512
NG = D // 128
W, DIL = 8, 2
HALO = 16
RB = 128
KR = HALO + RB
TICKS = 16
QSCALE = (DH ** -0.5) * 1.4426950408889634
NEG = -1e30
PST = 33

CFG = dict(BL=(0, 2, 8), NB=2, EC=16, EK=8, E0=0, EN=12, EL=8, OK=16, QO=0, CH=2, VK=2, LS=10, N0=84, NW=2, PS=3, LNK=28, PK=28, MK=6, MS=7)


def _nn(a, b):
    return jnp.dot(a, b, preferred_element_type=F32)


def _nt(a, b):
    return lax.dot_general(a, b, (((1,), (1,)), ((), ())), preferred_element_type=F32)


def _pk(x):
    return pltpu.bitcast(x.astype(BF16), I32)


def _up(x):
    return pltpu.bitcast(x, BF16)


def _blk(i, n=128):
    return slice(i * n, (i + 1) * n)


def _ds(i, n):
    return pl.ds(i * n if isinstance(i, int) else pl.multiple_of(i * n, n), n)


def _tiles(x):
    return [x[:, _blk(t)] for t in range(x.shape[1] // 128)]


def _fold8(x, op):
    return functools.reduce(op, [x[r:r + 8] for r in range(0, x.shape[0], 8)])


def _phi(t):
    return jnp.where(t > 0, t + 1.0, jnp.exp(t))


def _skew(xs):
    quarter = lax.broadcasted_iota(I32, xs[0].shape, 1) // DH
    for bit in (1, 2):
        xs = [jnp.where((quarter & bit) != 0, xs[i ^ bit], xs[i]) for i in range(4)]
    return xs


def _skew_rows(x):
    n = x.shape[0] // 4
    return jnp.concatenate(_skew([x[_blk(i, n)] for i in range(4)]), axis=0)


def _layernorm(load, init=None):
    tiles = _tiles(load(0))
    s = functools.reduce(jnp.add, tiles if init is None else [init] + tiles)
    m = jnp.sum(s, axis=-1, keepdims=True) * (1.0 / D)
    s = functools.reduce(jnp.add, [(x - m) * (x - m) for x in _tiles(load(1))])
    rs = lax.rsqrt(jnp.sum(s, axis=-1, keepdims=True) * (1.0 / D) + 1e-5)
    return _pk((load(2) - m) * rs)


class _Pacer:
    def __init__(self, z):
        self.z, self.sinks, self.side, self.slot = z, {}, {}, 0

    def zero(self, x):
        return (x if x.dtype == I32 else pltpu.bitcast(x, I32)) & self.z

    def sink(self, tick, x):
        zt = self.zero(x)
        self.sinks[tick] = self.sinks[tick] | zt if tick in self.sinks else zt

    def lhs(self, x):
        t0, self.slot = self.slot * TICKS, self.slot + 1
        cols = _tiles(x)
        for half in range(2):
            zts = [self.sinks.pop(t0 + half * 8 + r, None) for r in range(8)]
            if any(zt is not None for zt in zts):
                rows = [cols[4 * half][_blk(r, 8)] for r in range(8)]
                cols[4 * half] = jnp.concatenate(
                    [v if zt is None else v | zt for v, zt in zip(rows, zts)], axis=0)
        return _up(jnp.concatenate(cols, axis=1))

    def at(self, points, gen):
        next(gen)
        for p in points:
            self.side.setdefault(p, []).append(gen)

    def done(self, y):
        t0 = (self.slot - 1) * TICKS
        for v in range(TICKS):
            for gen in self.side.pop(t0 + v, []):
                now = t0 + (TICKS + v) // 2 + 7
                try:
                    gen.send((now, pltpu.bitcast(self.zero(y[_blk(v, 8)]), F32)))
                except StopIteration:
                    pass


def _kernel(x_hbm, wq_hbm, wk_hbm, wv_hbm, wo_hbm, beta_ref, wqkv_hbm, wob_hbm, out_ref,
            xin, wq, wk, wv, wo, wqkv, wob, wpt, wobp, pbuf, sems,
            xres, xna, obuf, gate, cmask, mt, zs, abufs, xm, xnb, ob2, qk_, vo, pb):
    NB, BL = CFG["NB"], CFG["BL"]
    NCH = len(BL) - 1
    it = pl.program_id(0)
    seg = it % NSEG
    nseg = (it + 1) % NSEG
    zz = [it // (2 * NSEG << n) for n in range(3)]
    z = zz[0]

    def a_copies(tr):
        cols = pl.ds(BL[tr] * 128, (BL[tr + 1] - BL[tr]) * 128)
        return [pltpu.make_async_copy(src.at[:, cols], dst.at[:, cols], sems.at[3 * tr + i])
                for i, (src, dst) in enumerate(((wk_hbm, wk), (wq_hbm, wq), (wv_hbm, wv)))]

    x0_copy = pltpu.make_async_copy(x_hbm.at[0:L], xin.at[0:L], sems.at[3 * NCH])
    late = [pltpu.make_async_copy(src, dst, sems.at[3 * NCH + 1 + i]) for i, (src, dst) in enumerate(
        ((wqkv_hbm, wqkv), (wob_hbm, wob), (wo_hbm, wo), (x_hbm.at[L:S], xin.at[L:S])))]

    @pl.when(it == 0)
    def _start():
        x0_copy.start()
        for c in a_copies(0):
            c.start()
        g = jax.nn.sigmoid(beta_ref[...].astype(F32).reshape(1, H))
        eye = lax.broadcasted_iota(I32, (H, H), 0) == lax.broadcasted_iota(I32, (H, H), 1)
        g = jnp.sum(jnp.where(eye, jnp.broadcast_to(g, (H, H)), 0.0), axis=1, keepdims=True)
        g = jnp.broadcast_to(g, (H, 128))
        for i in range(NG):
            gate[i] = g[_blk(i, 4)]
        cmask[...] = jnp.where(lax.broadcasted_iota(I32, (DH, 128), 0)
                               <= lax.broadcasted_iota(I32, (DH, 128), 1) % DH, 0.0, NEG)
        x0_copy.wait()

        def first_ln(i, carry):
            x = xin[_ds(i, RB), :].astype(F32)
            xres[z, _ds(i, RB), :] = x
            xna[_ds(i, RB // 2), :] = _layernorm(lambda p: xres[zz[p], _ds(i, RB), :] if p else x)
            return carry

        lax.fori_loop(0, L // RB, first_ln, 0)
        for c in [c for tr in range(1, NCH) for c in a_copies(tr)] + late:
            c.start()

    @pl.when(seg == 0)
    def _reset():
        mt[...] = jnp.zeros(mt.shape, F32)
        zs[...] = jnp.zeros(zs.shape, F32)
        qk_[0][0, :, 0:HALO, :] = jnp.zeros((NG, HALO, 128), F32)
        vo[0][0, :, 0:HALO, :] = jnp.zeros((NG, HALO, 128), F32)

    def a_trip(tr):
        @pl.when(it == 0)
        def _weights():
            for c in a_copies(tr):
                c.wait()

        U = BL[tr + 1] - BL[tr]
        pace = _Pacer(z)
        lane_head = lax.broadcasted_iota(I32, (128, 128), 1) // DH
        row_head = lax.broadcasted_iota(I32, (128, 128), 0) // DH

        def group(u):
            g = BL[tr] + u
            cols = _ds(g, 128)
            ks, pks, qms, pqs, vts, ss, pp, ams = abufs[u % 2]
            st = {}

            def proj(i, w):
                y = _nn(pace.lhs(xna[_blk(i, 64), :]), w[:, cols])
                pace.done(y)
                return y

            def proj_k(i):
                k = proj(i, wk)
                ks[z, _blk(i, 64), :] = _pk(k)
                pk = _phi(k)
                pks[z, _blk(i, 64), :] = _pk(pk)
                ps = _fold8(pk, jnp.add)
                st["pksum"] = ps if i == 0 else st["pksum"] + ps

            def proj_q(j):
                q = proj(j, wq)
                qj = _pk(q * QSCALE)
                for i in range(4):
                    for c in range(4):
                        qms[j][z, i, _blk(c, 16), :] = jnp.where(lane_head[:16] == c ^ i, qj[_blk(i, 16)], 0)
                pqs[z, _blk(j, 64), :] = _skew_rows(_pk(_phi(q)))

            def proj_v(i):
                vts[z, :, _blk(i)] = vt = pltpu.bitcast(proj(i, wv).astype(BF16).T, I32)
                deadline((pace.slot + CFG["VK"]) * TICKS, vt[56:])

            def deadline(tick, x):
                if tick < 12 * U * TICKS:
                    pace.sink(tick, x)

            def qk(j, i):
                n = j * 128 + (i + 1) * DH
                s = _nt(_up(ks[0, 0:n // 2, :]), _up(qms[j][0, i]))
                sd = s[n - DH:] + cmask[...]
                s = jnp.concatenate([s[:n - DH], sd], axis=0) if n > DH else sd
                ss[j][z, i, 16:16 + n, :] = s
                m = jnp.max(_fold8(s, jnp.maximum), axis=0, keepdims=True)
                ss[j][z, i, 0:8, :] = jnp.broadcast_to(m, (8, 128))

            def ex(plan):
                EC = CFG["EC"]
                for j in js:
                    n = (j + 1) * 128
                    l = [None] * 4
                    for r in range(0, n, EC):
                        tick, gated = next(plan)
                        zt = (yield)[1] if gated else None
                        if r == 0:
                            m = [ss[j][0, i, 0:8, :] for i in range(4)]
                        ps = [jnp.zeros((EC // 2, 128), I32)] * 4
                        for i in range(4):
                            if r < j * 128 + (i + 1) * DH:
                                m[i] = m[i] + zt if gated else m[i]
                                p = jnp.exp2(ss[j][0, i, 16 + r:16 + r + EC, :] - jnp.concatenate([m[i]] * (EC // 8)))
                                l[i] = _fold8(p, jnp.add) if r == 0 else l[i] + _fold8(p, jnp.add)
                                ps[i] = _pk(p)
                        ps = _skew(ps)
                        pp[j][z, 8 + r // 2:8 + (r + EC) // 2, :] = jnp.concatenate(ps, axis=1)
                        if r + EC == n:
                            l = [jnp.broadcast_to((1.0 - gate[g, h:h + 1, :]) / jnp.sum(v, axis=0, keepdims=True),
                                                  (8, 128)) for h, v in enumerate(_skew(l))]
                            pp[j][z, 0:8, :] = pltpu.bitcast(jnp.concatenate(l, axis=1), I32)
                        deadline(tick, ps[3][:8])
                        deadline(tick, functools.reduce(jnp.add, l))

            def mem():
                zm = jnp.where(lax.broadcasted_iota(I32, (16, 128), 0) == lane_head[:16],
                               jnp.broadcast_to(zs[g], (16, 128)), 0.0)
                r = _nt(jnp.concatenate([zm, mt[g]], axis=0).astype(BF16), _up(pqs[0]))
                inv = 1.0 / (r[0:8] + 1e-6)
                for h in range(4):
                    gh = jnp.concatenate([gate[g, h:h + 1, :]] * 4, axis=1)
                    ams[z, _blk(h, DH), :] = r[16 + h * DH:16 + (h + 1) * DH] * (gh * inv[h:h + 1])

            def pv(j):
                n = (j + 1) * 128
                outs = []
                for h in range(4):
                    o = _nn(_up(vts[0, _blk(h, DH // 2), 0:n]), _up(pp[j][0, 8:, _blk(h)]))
                    f = jnp.concatenate([pltpu.bitcast(pp[j][0, 0:8, _blk(h)], F32)] * 4, axis=0)
                    outs.append(o * f + ams[0, _blk(h, DH), _blk(j)])
                o = pltpu.bitcast(jnp.concatenate(outs, axis=0).astype(BF16).T, I32)
                obuf[_blk(j, 64), cols] = o = _skew_rows(o)
                deadline(pace.slot * TICKS + CFG['OK'] + 2 * j, functools.reduce(jnp.bitwise_or, [o[_blk(c, 8)] for c in range(8)]))

            def upd():
                mt[g] = new = mt[g] + jnp.where(lane_head == row_head, _nn(_up(vts[0]), _up(pks[0])), 0.0)
                deadline(pace.slot * TICKS + CFG['OK'], _fold8(new, jnp.add))
                zs[g] = zs[g] + jnp.sum(st["pksum"], axis=0, keepdims=True)

            js = (0, 1, 2, 3) if CFG["QO"] == 0 else (3, 2, 1, 0)

            def st_kq():
                for i in range(4):
                    proj_k(i)
                for j in js:
                    proj_q(j)

            def st_v():
                for i in range(4):
                    proj_v(i)

            def st_s():
                for j in js:
                    for i in (3, 2, 1, 0):
                        qk(j, i)
                n = 10 * 128 // CFG["EC"]
                span = (CFG["EN"] if u < U - 2 else CFG["EL"]) * TICKS - CFG["E0"]
                t0 = pace.slot * TICKS
                plan, points = [], []
                for c in range(n):
                    tick = CFG["E0"] + c * span // n
                    piece, half = divmod(tick - CFG["EK"] - 15, TICKS)
                    point = t0 + piece * TICKS + (TICKS - 1 if half >= 8 else 0)
                    gated = piece >= 0 and point not in points
                    plan.append((t0 + tick, gated))
                    if gated:
                        points.append(point)
                pace.at(points, ex(iter(plan)))

            def st_o():
                mem()
                for j in js:
                    pv(j)
                upd()

            return dict(kq=st_kq, v=st_v, s=st_s, o=st_o)

        order = [("kq", 0), ("s", 0)]
        for u in range(1, U - 1):
            order += [("kq", u), ("v", u - 1), ("s", u), ("o", u - 1)]
        order += [("kq", U - 1), ("s", U - 1), ("v", U - 2), ("v", U - 1), ("o", U - 2), ("o", U - 1)]
        gs = [group(u) for u in range(U)]
        for name, u in order:
            gs[u][name]()
        assert not pace.sinks and not pace.side

    with jax.named_scope("aloop"):
        for tr in range(NCH):
            a_trip(tr)

    def _prepare_b():
        def permute(t, buf, store):
            for h in range(H):
                buf[pl.ds(h, DH, stride=PST), :] = t[_blk(h, DH)]
            for d in range(DH):
                store(d, _pk(buf[pl.ds(d * PST, H), :]))

        with jax.named_scope('latewait'):
            for c in late:
                c.wait()

        def body(i, carry):
            for part in range(3):
                def store(d, v, part=part):
                    wpt[_blk(part * DH + d, H // 2), _ds(i, 128)] = v
                permute(wqkv[_ds(i, 128), _blk(part, D)].T.astype(F32), pbuf[part], store)

            def store_o(d, v):
                wobp[_blk(d, H // 2), _ds(i, 128)] = v
            permute(wob[:, _ds(i, 128)].astype(F32), pbuf[3], store_o)
            for s_ in range(1, NSEG):
                xres[s_, _ds(i, L // NG), :] = xin[_ds(s_ * NG + i, L // NG), :].astype(F32)
            return carry

        lax.fori_loop(0, NG, body, 0)

    with jax.named_scope("prep"):
        pl.when(it == 0)(_prepare_b)

    def r_trip(tr, carry):
        pace = _Pacer(z)

        def a_out(i, t):
            y = _nn(pace.lhs(obuf[_ds(tr * NB + i, RB // 2), :]), wo[:, _blk(t)])
            xm[i][z, :, _blk(t)] = xres[seg, _ds(tr * NB + i, RB), _blk(t)] + y
            return y

        def b_proj(i, part, t):
            y = _nt(pace.lhs(xnb[i][0]), _up(wpt[_blk(part * NG + t, 64), :]))
            if part == 0:
                qk_[i][z, t, KR:KR + RB, :] = y * QSCALE
            else:
                buf = (qk_, vo)[part - 1]
                buf[i][z, t, HALO:KR, :] = y
                if i + 1 < NB:
                    buf[i + 1][z, t, 0:HALO, :] = y[RB - HALO:]
            return y

        def b_out(i, t):
            x = xm[i][0, :, _blk(t)] + _nn(pace.lhs(ob2[i][0]), _up(wobp[:, _blk(t)]))
            xres[seg, _ds(tr * NB + i, RB), _blk(t)] = x
            out_ref[_ds(tr * NB + i, RB), _blk(t)] = x.astype(out_ref.dtype)
            return x

        def mid_ln(i):
            for r in range(RB // 16):
                now, zt = yield
                y = _layernorm(lambda p: xm[i][zz[p] if p else 0, _blk(r, 16), :], jnp.concatenate([zt, zt]))
                xnb[i][z, _blk(r, 8), :] = y
                pace.sink(now + CFG["LNK"], y[:, D - 128:])

        def next_ln():
            n = NB * RB // 16
            for r in range(n):
                now, zt = yield
                y = _layernorm(lambda p: xres[nseg + zz[p], _ds(tr * n + r, 16), :], jnp.concatenate([zt, zt]))
                xna[_ds(tr * n + r, 8), :] = y
                pace.sink(now + CFG["LNK"], y[:, D - 128:])

        def b_prob(i):
            for r in range(0, RB, 8):
                lg = []
                for w in range(W):
                    if w % CFG["NW"] == 0:
                        now, zt = yield
                    if w == 0:
                        q = [qk_[i][0, t, KR + r:KR + r + 8, :] for t in range(NG)]
                    a = zt
                    for t in range(NG):
                        a = a + q[t] * qk_[i][0, t, pl.ds(r + HALO - DIL * w, 8), :]
                    a = a + pltpu.roll(a, 64, 1)
                    a = a + pltpu.roll(a, 32, 1)
                    if i * RB + r < DIL * w:
                        pos = seg * L + tr * (NB * RB) + r + lax.broadcasted_iota(I32, (8, 128), 0)
                        a = jnp.where(pos >= DIL * w, a, NEG)
                    lg.append(a)
                m = functools.reduce(jnp.maximum, lg)
                e = [jnp.exp2(a - m) for a in lg]
                inv = 1.0 / functools.reduce(jnp.add, e)
                for w in range(W):
                    pb[i][z, w, r:r + 8, :] = p = e[w] * inv
                pace.sink(now + CFG["PK"], p)

        def b_mix(i):
            now, _ = yield
            for r in range(RB // 16):
                p = [pb[i][0, w, _blk(r, 16), :] for w in range(W)]
                for t in range(NG):
                    o = None
                    for c in range(4):
                        vv = vo[i][0, t, pl.ds(r * 16 + HALO - DIL * c - 8, 24), :]
                        for w, vw in ((c, vv[8:]), (c + 4, vv[:16])):
                            o = p[w] * vw if o is None else o + p[w] * vw
                    ob2[i][z, _blk(r, 8), _blk(t)] = o = _pk(o)
                    pace.sink(now + CFG["MK"] + (r * NG + t) * CFG["MS"] // 4, o)

        pt = functools.partial
        mxu = [pt(a_out, i, t) for i in range(NB) for t in range(NG)]
        mxu += [pt(b_proj, i, part, t) for i in range(NB) for part in range(2) for t in range(NG)]
        mxu += [pt(b_proj, i, 2, t) for i in range(NB) for t in range(NG)]
        mxu += [pt(b_out, i, t) for i in range(NB) for t in range(NG)]
        V = TICKS
        for i in range(NB):
            pace.at([V * (i + 1) * NG - 1 + n * CFG["LS"] for n in range(RB // 16)], mid_ln(i))
            s0 = V * (NB * NG + (i + 1) * 2 * NG)
            pace.at([s0 + n * CFG["PS"] for n in range(V * W // CFG["NW"])], b_prob(i))
            pace.at([V * (3 * NB * NG + (i + 1) * NG) - 1], b_mix(i))
        pace.at([V * NB * NG + CFG["N0"] + n * CFG["LS"] for n in range(NB * RB // 16)], next_ln())
        for f in mxu:
            pace.done(f())
        assert not pace.sinks and not pace.side
        for buf in (qk_, vo):
            buf[0][z, :, 0:HALO, :] = buf[NB - 1][0, :, RB:KR, :]
        return carry

    with jax.named_scope("rloop"):
        lax.fori_loop(0, L // (NB * RB), r_trip, 0)


@jax.jit
def pallas_interleave_layers__memory_aug_infini_attn__sliding_local_dilated__prompt_kernel(A_x, A_wq, A_wk, A_wv, A_wo, A_beta, B_x, B_wqkv, B_wo):
    del B_x
    any_spec = pl.BlockSpec(memory_space=pl.ANY)
    vmem = pltpu.VMEM
    NB = CFG["NB"]
    group_bufs = [
        vmem((1, L // 2, 128), I32),
        vmem((1, L // 2, 128), I32),
        [vmem((1, 4, 64, 128), I32)] * 4,
        vmem((1, L // 2, 128), I32),
        vmem((1, 64, L), I32),
        [vmem((1, 4, 128 * (j + 1) + 24, 128), F32) for j in range(4)],
        [vmem((1, 64 * (j + 1) + 8, 512), I32) for j in range(4)],
        vmem((1, 128, L), F32),
    ]
    out = pl.pallas_call(
        _kernel,
        grid=(2 * NSEG,),
        in_specs=[any_spec] * 5 + [pl.BlockSpec((H,), lambda i: (0,))] + [any_spec] * 2,
        out_specs=pl.BlockSpec((L, D), lambda i: (jnp.maximum(i - NSEG, 0), 0)),
        out_shape=jax.ShapeDtypeStruct((S, D), A_x.dtype),
        scratch_shapes=[
            vmem((S, D), BF16),
            vmem((D, D), BF16),
            vmem((D, D), BF16),
            vmem((D, D), BF16),
            vmem((D, D), BF16),
            vmem((D, 3 * D), BF16),
            vmem((D, D), BF16),
            vmem((3 * D // 2, D), I32),
            vmem((D // 2, D), I32),
            [vmem((DH * PST, 128), F32)] * 4,
            pltpu.SemaphoreType.DMA((3 * NG + 5,)),
            vmem((NSEG, L, D), F32),
            vmem((L // 2, D), I32),
            vmem((L // 2, D), I32),
            vmem((NG, 4, 128), F32),
            vmem((DH, 128), F32),
            vmem((NG, 128, 128), F32),
            vmem((NG, 1, 128), F32),
            [group_bufs] * 2,
            [vmem((1, RB, D), F32)] * NB,
            [vmem((1, RB // 2, D), I32)] * NB,
            [vmem((1, RB // 2, D), I32)] * NB,
            [vmem((1, NG, KR + RB + CFG.get("P1", 0), 128), F32)] * NB,
            [vmem((1, NG, KR + CFG.get("P2", 0), 128), F32)] * NB,
            [vmem((1, W, RB, 128), F32)] * NB,
        ],
        compiler_params=pltpu.CompilerParams(
            dimension_semantics=("arbitrary",), vmem_limit_bytes=110 * 1024 * 1024),
        name="fused_layers",
    )(A_x.reshape(S, D), A_wq, A_wk, A_wv, A_wo, A_beta, B_wqkv, B_wo)
    return out.reshape(A_x.shape)
```

```python
import functools

import jax
import jax.numpy as jnp
from jax import lax
import jax.experimental.pallas as pl
import jax.experimental.pallas.tpu as pltpu

F32 = jnp.float32
BF16 = jnp.bfloat16
I32 = jnp.int32

S, D, H, DH = 2048, 1024, 32, 32
NSEG, L = 4, 512
NG = D // 128
W, DIL = 8, 2
HALO = 16
RB = 128
KR = HALO + RB
TICKS = 16
QSCALE = (DH ** -0.5) * 1.4426950408889634
NEG = -1e30
PST = 36

CFG = dict(BL=(0, 2, 8), NB=2, EC=16, EK=14, FK=4, PU=2, WT=dict(kq=1, v=1, s=1, o=0), OK=24, JS=(0, 1, 2, 3), J0=(3, 2, 1, 0), GJ=1, CH=2, VK=24, LS=10, N0=84, NW=2, PS=(6, 4), D2=1, ALL=0, CUT=4, DEF=1, N1=16, NS=10, LNK=28, PK=28, MK=6, MS=7)


def _nn(a, b):
    return jnp.dot(a, b, preferred_element_type=F32)


def _nt(a, b):
    return lax.dot_general(a, b, (((1,), (1,)), ((), ())), preferred_element_type=F32)


def _pk(x):
    return pltpu.bitcast(x.astype(BF16), I32)


def _pk2(a, b):
    return _tiles(_pk(jnp.concatenate([a, b], axis=1)))


def _up(x):
    return pltpu.bitcast(x, BF16)


def _blk(i, n=128):
    return slice(i * n, (i + 1) * n)


def _ds(i, n):
    return pl.ds(i * n if isinstance(i, int) else pl.multiple_of(i * n, n), n)


def _tiles(x):
    return [x[:, _blk(t)] for t in range(x.shape[1] // 128)]


def _fold8(x, op):
    return functools.reduce(op, [x[r:r + 8] for r in range(0, x.shape[0], 8)])


def _phi(t):
    return jnp.where(t > 0, t + 1.0, jnp.exp(t))


def _skew(xs):
    quarter = lax.broadcasted_iota(I32, xs[0].shape, 1) // DH
    for bit in (1, 2):
        xs = [jnp.where((quarter & bit) != 0, xs[i ^ bit], xs[i]) for i in range(4)]
    return xs


def _skew_rows(x):
    n = x.shape[0] // 4
    return jnp.concatenate(_skew([x[_blk(i, n)] for i in range(4)]), axis=0)


def _layernorm(load, init=None):
    tiles = _tiles(load(0))
    s = functools.reduce(jnp.add, tiles if init is None else [init] + tiles)
    m = jnp.sum(s, axis=-1, keepdims=True) * (1.0 / D)
    s = functools.reduce(jnp.add, [(x - m) * (x - m) for x in _tiles(load(1))])
    rs = lax.rsqrt(jnp.sum(s, axis=-1, keepdims=True) * (1.0 / D) + 1e-5)
    return _pk((load(2) - m) * rs)


class _Pacer:
    def __init__(self, z):
        self.z, self.sinks, self.side, self.now = z, {}, {}, 0

    def zero(self, x):
        return (x if x.dtype == I32 else pltpu.bitcast(x, I32)) & self.z

    def sink(self, tick, x):
        assert tick >= self.now
        zt = self.zero(x)
        self.sinks[tick] = self.sinks[tick] | zt if tick in self.sinks else zt

    def lhs(self, x):
        cols = _tiles(x)
        n = x.shape[0] // 8
        for c in range(0, len(cols), 4):
            zts = [self.sinks.pop(self.now + r, None) for r in range(n)]
            self.now += n
            if any(zt is not None for zt in zts):
                rows = [cols[c][_blk(r, 8)] for r in range(n)]
                cols[c] = jnp.concatenate([v if zt is None else v | zt for v, zt in zip(rows, zts)])
        return _up(jnp.concatenate(cols, axis=1))

    def at(self, points, gen):
        next(gen, None)
        for p in points:
            self.side.setdefault(p, []).append(gen)

    def done(self, y):
        t0 = self.now - TICKS
        for v in range(TICKS):
            for gen in self.side.pop(t0 + v, []):
                tick = t0 + (TICKS + v) // 2 + 7
                try:
                    gen.send((tick, pltpu.bitcast(self.zero(y[_blk(v, 8)]), F32)))
                except StopIteration:
                    pass


def _kernel(x_hbm, wq_hbm, wk_hbm, wv_hbm, wo_hbm, beta_ref, wqkv_hbm, wob_hbm, out_ref,
            xin, wq, wk, wv, wo, wqkv, wob, wpt, wobp, pbuf, sems,
            xres, xcur, stage, xout, xna, obuf, gate, cmask, mt, zs, abufs, xm, xnb, ob2, qk_, vo, pb):
    NB, BL = CFG["NB"], CFG["BL"]
    NCH = len(BL) - 1
    it = pl.program_id(0)
    seg = it % NSEG
    nseg = (it + 1) % NSEG
    zz = [it // (2 * NSEG << n) for n in range(3)]
    z = zz[0]

    def a_copies(tr):
        cols = pl.ds(BL[tr] * 128, (BL[tr + 1] - BL[tr]) * 128)
        return [pltpu.make_async_copy(src.at[:, cols], dst.at[:, cols], sems.at[3 * tr + i])
                for i, (src, dst) in enumerate(((wk_hbm, wk), (wq_hbm, wq), (wv_hbm, wv)))]

    x0_copy = pltpu.make_async_copy(x_hbm.at[0:L], xin.at[0:L], sems.at[3 * NCH])
    late = [pltpu.make_async_copy(src, dst, sems.at[3 * NCH + 1 + i]) for i, (src, dst) in enumerate(
        ((wqkv_hbm, wqkv), (wob_hbm, wob), (wo_hbm, wo), (x_hbm.at[L:S], xin.at[L:S])))]

    def _start():
        x0_copy.start()
        for c in a_copies(0):
            c.start()
        g = jax.nn.sigmoid(beta_ref[...].astype(F32).reshape(1, H))
        eye = lax.broadcasted_iota(I32, (H, H), 0) == lax.broadcasted_iota(I32, (H, H), 1)
        g = jnp.sum(jnp.where(eye, jnp.broadcast_to(g, (H, H)), 0.0), axis=1, keepdims=True)
        g = jnp.broadcast_to(g, (H, 128))
        for i in range(NG):
            gate[i] = jnp.concatenate([g[_blk(i, 4)]] * 2)
        cmask[...] = jnp.where(lax.broadcasted_iota(I32, (DH, 128), 0)
                               <= lax.broadcasted_iota(I32, (DH, 128), 1) % DH, 0.0, NEG)
        x0_copy.wait()

        def first_ln(i, carry):
            x = xin[_ds(i, RB), :].astype(F32)
            xcur[_ds(i, RB), :] = x
            xna[_ds(i, RB // 2), :] = _layernorm(lambda p: xcur[_ds(i + zz[p], RB), :] if p else x)
            return carry

        lax.fori_loop(0, L // RB, first_ln, 0)
        for c in [c for tr in range(1, NCH) for c in a_copies(tr)] + late:
            c.start()

    with jax.named_scope('start'):
        pl.when(it == 0)(_start)

    @pl.when(seg == 0)
    def _reset():
        mt[...] = jnp.zeros(mt.shape, F32)
        zs[...] = jnp.zeros(zs.shape, F32)
        qk_[0][0, :, 0:HALO, :] = jnp.zeros((NG, HALO, 128), F32)
        vo[0][0, :, 0:HALO, :] = jnp.zeros((NG, HALO, 128), F32)

    def a_trip(tr):
        @pl.when(it == 0)
        def _weights():
            for c in a_copies(tr):
                c.wait()

        U = BL[tr + 1] - BL[tr]
        LEN = dict(kq=8 * TICKS, v=4 * TICKS, s=80, o=0)
        order = [("kq", 0), ("s", 0)]
        for u in range(1, U - 1):
            order += [("kq", u), ("v", u - 1), ("s", u), ("o", u - 1)]
        order += [("kq", U - 1), ("s", U - 1), ("v", U - 2), ("v", U - 1), ("o", U - 2), ("o", U - 1)]
        pace = _Pacer(z)
        lane_head = lax.broadcasted_iota(I32, (128, 128), 1) // DH
        row_head = lax.broadcasted_iota(I32, (128, 128), 0) // DH

        def group(u):
            g = BL[tr] + u
            cols = _ds(g, 128)
            ks, pks, qms, pqs, vts, ss, pp, fs, ams = abufs[u % 2]
            st = {}

            def proj(i, w):
                y = _nn(pace.lhs(xna[_blk(i, 64), :]), w[:, cols])
                pace.done(y)
                return y

            def proj_k(i):
                k = proj(i, wk)
                pk = _phi(k)
                ks[z, _blk(i, 64), :], pks[z, _blk(i, 64), :] = _pk2(k, pk)
                ps = _fold8(pk, jnp.add)
                st["pksum"] = ps if i == 0 else st["pksum"] + ps

            def proj_q(j):
                q = proj(j, wq)
                qj, pq = _pk2(q * QSCALE, _phi(q))
                for i in range(4):
                    for c in range(4):
                        qms[j][z, i, _blk(c, 16), :] = jnp.where(lane_head[:16] == c ^ i, qj[_blk(i, 16)], 0)
                pqs[z, _blk(j, 64), :] = _skew_rows(pq)

            def proj_v(i):
                vts[z, :, _blk(i)] = vt = pltpu.bitcast(proj(i, wv).astype(BF16).T, I32)
                deadline(pace.now + CFG["VK"], vt[56:])

            def deadline(tick, x):
                if tick < U * sum(LEN.values()):
                    pace.sink(tick, x)

            def qk(j, i):
                n = j * 128 + (i + 1) * DH
                s = _nt((pace.lhs if i == 3 else _up)(ks[0, 0:n // 2, :]), _up(qms[j][0, i]))
                sd = s[n - DH:] + cmask[...]
                s = jnp.concatenate([s[:n - DH], sd], axis=0) if n > DH else sd
                ss[j][z, i, 16:16 + n, :] = s
                m = jnp.max(_fold8(s, jnp.maximum), axis=0, keepdims=True)
                ss[j][z, i, 0:8, :] = st['m', j] = jnp.broadcast_to(m, (8, 128))

            def ex(plan):
                EC = CFG["EC"]
                zt = pltpu.bitcast(pace.zero(st['m', js[CFG['GJ']]]), F32)
                for j in js:
                    n = (j + 1) * 128
                    l = [None] * 4
                    for r in range(0, n, EC):
                        tick, gated = next(plan)
                        zt = (yield)[1] if gated else zt
                        if r == 0:
                            m = [ss[j][0, i, 0:8, :] for i in range(4)]
                        ps = []
                        for i in range(4):
                            if r < j * 128 + (i + 1) * DH:
                                m[i] = m[i] + zt if gated or r == 0 else m[i]
                                p = jnp.exp2(ss[j][0, i, 16 + r:16 + r + EC, :] - jnp.concatenate([m[i]] * (EC // 8)))
                                l[i] = _fold8(p, jnp.add) if r == 0 else l[i] + _fold8(p, jnp.add)
                                ps.append(p)
                        ps = _skew([jnp.zeros((EC // 2, 128), I32)] * (4 - len(ps)) + _tiles(_pk(jnp.concatenate(ps, axis=1))))
                        pp[j][z, r // 2:(r + EC) // 2, :] = jnp.concatenate(ps, axis=1)
                        deadline(tick + CFG["D2"], (ps[0] | ps[1] | ps[2] | ps[3])[:8] if CFG["ALL"] else ps[3][:8])
                        deadline(tick, (l[0] + l[1]) + (l[2] + l[3]))
                    row = lax.broadcasted_iota(I32, (8, 128), 0)
                    tot = jnp.ones((8, 128), F32)
                    for h, v in enumerate(_skew(l)):
                        tot = jnp.where(row == h, jnp.sum(v, axis=0, keepdims=True), tot)
                    fs[z, j] = f = (1.0 - gate[g]) / tot
                    deadline(tick + CFG["FK"], f)

            def mem():
                zm = jnp.where(lax.broadcasted_iota(I32, (16, 128), 0) == lane_head[:16],
                               jnp.broadcast_to(zs[g], (16, 128)), 0.0)
                r = _nt(jnp.concatenate([zm, mt[g]], axis=0).astype(BF16), _up(pqs[0]))
                f = jnp.concatenate([gate[g]] * 4, axis=1) / (r[0:8] + 1e-6)
                for h in range(4):
                    ams[z, _blk(h, DH), :] = r[16 + h * DH:16 + (h + 1) * DH] * f[h:h + 1]

            def pv(j):
                n = (j + 1) * 128
                outs = []
                for h in range(4):
                    o = _nn(_up(vts[0, _blk(h, DH // 2), 0:n]), _up(pp[j][0, :, _blk(h)]))
                    f = fs[0, j, h:h + 1, :]
                    outs.append(o * f + ams[0, _blk(h, DH), _blk(j)])
                o = pltpu.bitcast(jnp.concatenate(outs, axis=0).astype(BF16).T, I32)
                obuf[_blk(j, 64), cols] = o = _skew_rows(o)
                deadline(pace.now + CFG['OK'] + 2 * j, functools.reduce(jnp.bitwise_or, [o[_blk(c, 8)] for c in range(8)]))

            def upd():
                mt[g] = new = mt[g] + jnp.where(lane_head == row_head, _nn(_up(vts[0]), _up(pks[0])), 0.0)
                deadline(pace.now + CFG['OK'], _fold8(new, jnp.add))
                zs[g] = zs[g] + jnp.sum(st["pksum"], axis=0, keepdims=True)

            js = CFG["JS"]

            def st_kq():
                for i in range(4):
                    proj_k(i)
                for j in js:
                    proj_q(j)

            def st_v():
                for i in range(4):
                    proj_v(i)

            def st_s():
                for j in js:
                    for i in (CFG['J0'] if j == 0 else (3, 2, 1, 0)):
                        qk(j, i)
                n = 10 * 128 // CFG["EC"]
                i0 = order.index(("s", u)) + 1
                i1 = order.index(("s", u + 1)) + 1 if u + 1 < U else len(order)
                slots, starts, t = [], [], pace.now
                for name, _ in order[i0:i1]:
                    slots += [t + d for d in range(LEN[name]) for _ in range(CFG["WT"][name])]
                    if name != "s":
                        starts += list(range(t, t + LEN[name], TICKS))
                    t += LEN[name]
                slots = slots[:len(slots) - CFG['CUT']]
                plan, points = [], []
                for c in range(n):
                    tick = slots[c * len(slots) // n]
                    cand = [p + v for p in starts for v in (0, TICKS - 1)
                            if p + (TICKS + v) // 2 + 7 + CFG["EK"] <= tick]
                    gated = bool(cand) and cand[-1] not in points
                    plan.append((tick, gated))
                    if gated:
                        points.append(cand[-1])
                pace.at(points, ex(iter(plan)))

            def st_o():
                mem()
                for j in js:
                    pv(j)
                upd()

            return dict(kq=st_kq, v=st_v, s=st_s, o=st_o)

        gs = [group(u) for u in range(U)]
        for name, u in order:
            gs[u][name]()
        assert not pace.sinks and not pace.side

    with jax.named_scope("aloop"):
        for tr in range(NCH):
            a_trip(tr)

    def _prepare_b():
        def permute(t, buf, store):
            for h in range(H):
                buf[pl.ds(h, DH, stride=PST), :] = t[_blk(h, DH)]
            for d in range(DH):
                store(d, _pk(buf[pl.ds(d * PST, H), :]))

        with jax.named_scope('latewait'):
            for c in late:
                c.wait()

        def body(n, carry):
            for u in range(CFG["PU"]):
                i = n * CFG["PU"] + u
                ts = [wqkv[_ds(i, 128), _blk(part, D)].T for part in range(3)]

                def store_o(d, v):
                    wobp[_blk(d, H // 2), _ds(i, 128)] = v
                permute(wob[:, _ds(i, 128)].astype(F32), pbuf[3], store_o)
                for part in range(3):
                    def store(d, v):
                        wpt[_blk(part * DH + d, H // 2), _ds(i, 128)] = v
                    permute(ts[part].astype(F32), pbuf[part], store)
            return carry

        lax.fori_loop(0, NG // CFG["PU"], body, 0)

    with jax.named_scope("prep"):
        pl.when(it == 0)(_prepare_b)

    NR = L // (NB * RB)

    def out_copy(tr):
        return pltpu.make_async_copy(xout.at[_ds(tr, NB * RB)], out_ref.at[_ds(seg * NR + tr, NB * RB)],
                                     sems.at[3 * NCH + 5 + tr])

    def r_trip(tr, carry):
        pl.when(it > NSEG)(out_copy(tr).wait)
        pace = _Pacer(z)

        def a_out(i, t):
            y = _nn(pace.lhs(obuf[_ds(tr * NB + i, RB // 2), :]), wo[:, _blk(t)])
            xm[i][z, :, _blk(t)] = xcur[_ds(tr * NB + i, RB), _blk(t)] + y
            return y

        def b_proj(i, part, t):
            y = _nt(pace.lhs(xnb[i][0]), _up(wpt[_blk(part * NG + t, 64), :]))
            if part == 0:
                qk_[i][z, t, KR:KR + RB, :] = y * QSCALE
            else:
                buf = (qk_, vo)[part - 1]
                buf[i][z, t, HALO:KR, :] = y
                if i + 1 < NB:
                    buf[i + 1][z, t, 0:HALO, :] = y[RB - HALO:]
            return y

        def b_out(i, t):
            x = xm[i][0, :, _blk(t)] + _nn(pace.lhs(ob2[i][0]), _up(wobp[:, _blk(t)]))
            xres[seg, _ds(tr * NB + i, RB), _blk(t)] = x
            xout[_ds(tr * NB + i, RB), _blk(t)] = x.astype(BF16)
            return x

        def mid_ln(i):
            for r in range(RB // 16):
                now, zt = yield
                y = _layernorm(lambda p: xm[i][zz[p] if p else 0, _blk(r, 16), :], jnp.concatenate([zt, zt]))
                xnb[i][z, _blk(r, 8), :] = y
                pace.sink(now + CFG["LNK"], y[:, D - 128:])

        def next_ln():
            n = NB * RB // 16
            for r in range(n):
                now, zt = yield
                rows = _ds(tr * n + r, 16)

                def load(p):
                    if p:
                        return stage[r % 3][zz[p]]
                    x = xin[_ds(nseg * (L // 16) + tr * n + r, 16), :].astype(F32)
                    x = jnp.where(it < NSEG - 1, x, xres[nseg, rows, :])
                    stage[r % 3][z] = x
                    xcur[rows, :] = x
                    return x

                y = _layernorm(load, jnp.concatenate([zt, zt]))
                xna[_ds(tr * n + r, 8), :] = y
                pace.sink(now + CFG["LNK"], y[:, D - 128:])

        def b_prob(i):
            for r in range(0, RB, 8):
                lg = []
                for w in range(W):
                    if w % CFG["NW"] == 0:
                        now, zt = yield
                    if w == 0:
                        q = [qk_[i][0, t, KR + r:KR + r + 8, :] for t in range(NG)]
                    a = zt
                    for t in range(NG):
                        a = a + q[t] * qk_[i][0, t, pl.ds(r + HALO - DIL * w, 8), :]
                    a = a + pltpu.roll(a, 64, 1)
                    a = a + pltpu.roll(a, 32, 1)
                    if i * RB + r < DIL * w:
                        pos = seg * L + tr * (NB * RB) + r + lax.broadcasted_iota(I32, (8, 128), 0)
                        a = jnp.where(pos >= DIL * w, a, NEG)
                    lg.append(a)
                m = functools.reduce(jnp.maximum, lg)
                e = [jnp.exp2(a - m) for a in lg]
                tot = functools.reduce(jnp.add, e)
                if CFG["DEF"]:
                    for w, p in enumerate(e + [tot]):
                        pb[i][z, w, r:r + 8, :] = p
                else:
                    inv = 1.0 / tot
                    for w in range(W):
                        pb[i][z, w, r:r + 8, :] = p = e[w] * inv
                pace.sink(now + CFG["PK"], p)

        def b_mix(i):
            now, _ = yield
            for r in range(RB // 16):
                p = [pb[i][0, w, _blk(r, 16), :] for w in range(W)]
                if CFG["DEF"]:
                    inv = 1.0 / pb[i][0, W, _blk(r, 16), :]
                for t in range(NG):
                    o = None
                    for c in range(4):
                        vv = vo[i][0, t, pl.ds(r * 16 + HALO - DIL * c - 8, 24), :]
                        for w, vw in ((c, vv[8:]), (c + 4, vv[:16])):
                            o = p[w] * vw if o is None else o + p[w] * vw
                    ob2[i][z, _blk(r, 8), _blk(t)] = o = _pk(o * inv if CFG["DEF"] else o)
                    pace.sink(now + CFG["MK"] + (r * NG + t) * CFG["MS"] // 4, o)

        def carry_halo():
            for buf in (qk_, vo):
                _, zt = yield
                buf[0][z, :, 0:HALO, :] = buf[NB - 1][0, :, RB:KR, :] + jnp.concatenate([zt, zt])

        pace.at([TICKS * ((5 * NB - 1) * NG + n) for n in (5, 6)], carry_halo())
        pt = functools.partial
        mxu = [pt(a_out, i, t) for i in range(NB) for t in range(NG)]
        mxu += [pt(b_proj, i, part, t) for i in range(NB) for part in range(2) for t in range(NG)]
        mxu += [pt(b_proj, i, 2, t) for i in range(NB) for t in range(NG)]
        mxu += [pt(b_out, i, t) for i in range(NB) for t in range(NG)]
        V = TICKS
        for i in range(NB):
            pace.at([V * (i + 1) * NG - 1 + n * CFG["LS"] for n in range(RB // 16)], mid_ln(i))
            s0 = V * (NB * NG + (i + 1) * 2 * NG)
            pace.at([s0 + n * CFG["PS"][i] // 2 for n in range(V * W // CFG["NW"])], b_prob(i))
            pace.at([V * (3 * NB * NG + (i + 1) * NG) - 1], b_mix(i))
        n1 = CFG["N1"]
        pace.at([V * NB * NG + CFG["N0"] + n * CFG["NS"] for n in range(n1)]
                + [V * (5 * NB - 1) * NG + n * CFG["LS"] - 1 for n in range(NB * RB // 16 - n1)], next_ln())
        for f in mxu:
            pace.done(f())
        assert not pace.sinks and not pace.side
        pl.when(it >= NSEG)(out_copy(tr).start)
        return carry

    with jax.named_scope("rloop"):
        lax.fori_loop(0, NR, r_trip, 0)

    @pl.when(it == 2 * NSEG - 1)
    def _finish():
        for tr in range(NR):
            out_copy(tr).wait()


@jax.jit
def pallas_interleave_layers__memory_aug_infini_attn__sliding_local_dilated__prompt_kernel(A_x, A_wq, A_wk, A_wv, A_wo, A_beta, B_x, B_wqkv, B_wo):
    del B_x
    any_spec = pl.BlockSpec(memory_space=pl.ANY)
    vmem = pltpu.VMEM
    NB = CFG["NB"]
    group_bufs = [
        vmem((1, L // 2, 128), I32),
        vmem((1, L // 2, 128), I32),
        [vmem((1, 4, 64, 128), I32)] * 4,
        vmem((1, L // 2, 128), I32),
        vmem((1, 64, L), I32),
        [vmem((1, 4, 128 * (j + 1) + 24, 128), F32) for j in range(4)],
        [vmem((1, 64 * (j + 1), 512), I32) for j in range(4)],
        vmem((1, 4, 8, 128), F32),
        vmem((1, 128, L), F32),
    ]
    out = pl.pallas_call(
        _kernel,
        grid=(2 * NSEG,),
        in_specs=[any_spec] * 5 + [pl.BlockSpec((H,), lambda i: (0,))] + [any_spec] * 2,
        out_specs=any_spec,
        out_shape=jax.ShapeDtypeStruct((S, D), A_x.dtype),
        scratch_shapes=[
            vmem((S, D), BF16),
            vmem((D, D), BF16),
            vmem((D, D), BF16),
            vmem((D, D), BF16),
            vmem((D, D), BF16),
            vmem((D, 3 * D), BF16),
            vmem((D, D), BF16),
            vmem((3 * D // 2, D), I32),
            vmem((D // 2, D), I32),
            [vmem((DH * PST, 128), F32)] * 4,
            pltpu.SemaphoreType.DMA((3 * NG + 5,)),
            vmem((NSEG, L, D), F32),
            vmem((L, D), F32),
            [vmem((1, 16, D), F32)] * 3,
            vmem((L, D), BF16),
            vmem((L // 2, D), I32),
            vmem((L // 2, D), I32),
            vmem((NG, 8, 128), F32),
            vmem((DH, 128), F32),
            vmem((NG, 128, 128), F32),
            vmem((NG, 1, 128), F32),
            [group_bufs] * 2,
            [vmem((1, RB, D), F32)] * NB,
            [vmem((1, RB // 2, D), I32)] * NB,
            [vmem((1, RB // 2, D), I32)] * NB,
            [vmem((1, NG, KR + RB + CFG.get("P1", 0), 128), F32)] * NB,
            [vmem((1, NG, KR + CFG.get("P2", 0), 128), F32)] * NB,
            [vmem((1, W + 1, RB + CFG.get('P3', 0), 128), F32)] * NB,
        ],
        compiler_params=pltpu.CompilerParams(
            dimension_semantics=("arbitrary",), vmem_limit_bytes=110 * 1024 * 1024),
        name="fused_layers",
    )(A_x.reshape(S, D), A_wq, A_wk, A_wv, A_wo, A_beta, B_wqkv, B_wo)
    return out.reshape(A_x.shape)
```

```python
import functools

import jax
import jax.numpy as jnp
from jax import lax
import jax.experimental.pallas as pl
import jax.experimental.pallas.tpu as pltpu

F32 = jnp.float32
BF16 = jnp.bfloat16
I32 = jnp.int32

S, D, H, DH = 2048, 1024, 32, 32
NSEG, L = 4, 512
NG = D // 128
W, DIL = 8, 2
HALO = 16
RB = 128
KR = HALO + RB
TICKS = 16
QSCALE = (DH ** -0.5) * 1.4426950408889634
NEG = -1e30
PST = 68

CFG = dict(BL=(0, 2, 8), NB=2, EC=16, EK=10, FK=4, PU=2, WT=dict(kq=1, v=1, s=1, o=0, m=1), OL=12, WW=1, OK=24, JS=(0, 1, 2, 3), J0=(3, 2, 1, 0), GJ=1, CH=2, VK=24, LS=10, N0=84, NW=2, PS=(6, 4), D2=1, ALL=0, CUT=4, DEF=1, N1=16, NS=10, LNK=28, PK=28, MK=6, MS=7)


def _nn(a, b):
    return jnp.dot(a, b, preferred_element_type=F32)


def _nt(a, b):
    return lax.dot_general(a, b, (((1,), (1,)), ((), ())), preferred_element_type=F32)


def _pk(x):
    return pltpu.bitcast(x.astype(BF16), I32)


def _pk2(a, b):
    return _tiles(_pk(jnp.concatenate([a, b], axis=1)))


def _up(x):
    return pltpu.bitcast(x, BF16)


def _blk(i, n=128):
    return slice(i * n, (i + 1) * n)


def _ds(i, n):
    return pl.ds(i * n if isinstance(i, int) else pl.multiple_of(i * n, n), n)


def _tiles(x):
    return [x[:, _blk(t)] for t in range(x.shape[1] // 128)]


def _fold8(x, op):
    return functools.reduce(op, [x[r:r + 8] for r in range(0, x.shape[0], 8)])


def _phi(t):
    return jnp.where(t > 0, t + 1.0, jnp.exp(t))


def _skew(xs):
    quarter = lax.broadcasted_iota(I32, xs[0].shape, 1) // DH
    for bit in (1, 2):
        xs = [jnp.where((quarter & bit) != 0, xs[i ^ bit], xs[i]) for i in range(4)]
    return xs


def _skew_rows(x):
    n = x.shape[0] // 4
    return jnp.concatenate(_skew([x[_blk(i, n)] for i in range(4)]), axis=0)


def _layernorm(load, init=None):
    tiles = _tiles(load(0))
    s = functools.reduce(jnp.add, tiles if init is None else [init] + tiles)
    m = jnp.sum(s, axis=-1, keepdims=True) * (1.0 / D)
    s = functools.reduce(jnp.add, [(x - m) * (x - m) for x in _tiles(load(1))])
    rs = lax.rsqrt(jnp.sum(s, axis=-1, keepdims=True) * (1.0 / D) + 1e-5)
    return _pk((load(2) - m) * rs)


class _Pacer:
    def __init__(self, z):
        self.z, self.sinks, self.side, self.now = z, {}, {}, 0

    def zero(self, x):
        return (x if x.dtype == I32 else pltpu.bitcast(x, I32)) & self.z

    def sink(self, tick, x):
        assert tick >= self.now
        zt = self.zero(x)
        self.sinks[tick] = self.sinks[tick] | zt if tick in self.sinks else zt

    def lhs(self, x):
        cols = _tiles(x)
        n = x.shape[0] // 8
        for c in range(0, len(cols), 4):
            zts = [self.sinks.pop(self.now + r, None) for r in range(n)]
            self.now += n
            if any(zt is not None for zt in zts):
                rows = [cols[c][_blk(r, 8)] for r in range(n)]
                cols[c] = jnp.concatenate([v if zt is None else v | zt for v, zt in zip(rows, zts)])
        return _up(jnp.concatenate(cols, axis=1))

    def at(self, points, gen):
        next(gen, None)
        for p in points:
            self.side.setdefault(p, []).append(gen)

    def done(self, y):
        t0 = self.now - TICKS
        for v in range(TICKS):
            for gen in self.side.pop(t0 + v, []):
                tick = t0 + (TICKS + v) // 2 + 7
                try:
                    gen.send((tick, pltpu.bitcast(self.zero(y[_blk(v, 8)]), F32)))
                except StopIteration:
                    pass


def _kernel(x_hbm, wq_hbm, wk_hbm, wv_hbm, wo_hbm, beta_hbm, wqkv_hbm, wob_hbm, out_ref,
            xin, wq, wk, wv, wo, wqkv, wob, beta, wa, wb, sems,
            xres, xcur, stage, xout, xna, obuf, gate, cmask, mt, zs, abufs, xm, xnb, ob2, qk_, vo, pb):
    NB, BL = CFG["NB"], CFG["BL"]
    NCH = len(BL) - 1
    it = pl.program_id(0)
    seg = it % NSEG
    nseg = (it + 1) % NSEG
    zz = [it // (2 * NSEG << n) for n in range(3)]
    z = zz[0]
    last = lambda cond: z

    def a_copies(tr):
        cols = pl.ds(BL[tr] * 128, (BL[tr + 1] - BL[tr]) * 128)
        return [pltpu.make_async_copy(src.at[:, cols], dst.at[:, cols], sems.at[3 * tr + i])
                for i, (src, dst) in enumerate(((wk_hbm, wk), (wq_hbm, wq), (wv_hbm, wv)))]

    x0_copy = pltpu.make_async_copy(x_hbm.at[0:L], xin.at[0:L], sems.at[3 * NCH])
    late = [pltpu.make_async_copy(src, dst, sems.at[3 * NCH + 1 + i]) for i, (src, dst) in enumerate(
        ((wqkv_hbm, wqkv), (wob_hbm, wob), (wo_hbm, wo), (x_hbm.at[L:S], xin.at[L:S])))]

    def _start():
        beta_copy = pltpu.make_async_copy(beta_hbm, beta, sems.at[3 * NCH + 7])
        beta_copy.start()
        x0_copy.start()
        for c in a_copies(0):
            c.start()

        def clear(i, carry):
            xres[1:, _ds(i, 32), :] = jnp.zeros((NSEG - 1, 32, D), F32)
            return carry

        lax.fori_loop(0, L // 32, clear, 0)
        beta_copy.wait()
        g = jax.nn.sigmoid(beta[...].astype(F32).reshape(1, H))
        eye = lax.broadcasted_iota(I32, (H, H), 0) == lax.broadcasted_iota(I32, (H, H), 1)
        g = jnp.sum(jnp.where(eye, jnp.broadcast_to(g, (H, H)), 0.0), axis=1, keepdims=True)
        g = jnp.broadcast_to(g, (H, 128))
        for i in range(NG):
            gate[i] = jnp.concatenate([g[_blk(i, 4)]] * 2)
        cmask[...] = jnp.where(lax.broadcasted_iota(I32, (DH, 128), 0)
                               <= lax.broadcasted_iota(I32, (DH, 128), 1) % DH, 0.0, NEG)
        x0_copy.wait()

        def first_ln(i, carry):
            x = xin[_ds(i, RB), :].astype(F32)
            xcur[_ds(i, RB), :] = x
            xna[_ds(i, RB // 2), :] = _layernorm(lambda p: xcur[_ds(i + zz[p], RB), :] if p else x)
            return carry

        lax.fori_loop(0, L // RB, first_ln, 0)
        for c in [c for tr in range(1, NCH) for c in a_copies(tr)] + late:
            c.start()

    with jax.named_scope('start'):
        pl.when(it == 0)(_start)

    @pl.when(seg == 0)
    def _reset():
        mt[...] = jnp.zeros(mt.shape, F32)
        zs[...] = jnp.zeros(zs.shape, F32)
        qk_[0][0, :, 0:HALO, :] = jnp.zeros((NG, HALO, 128), F32)
        vo[0][0, :, 0:HALO, :] = jnp.zeros((NG, HALO, 128), F32)

    def a_trip(tr):
        @pl.when(it == 0)
        def _weights():
            for c, src, dst in zip(a_copies(tr), (wk, wq, wv), wa):
                c.wait()
                if CFG["WW"]:
                    cols = slice(BL[tr] * 128, BL[tr + 1] * 128)

                    def body(i, carry, src=src, dst=dst):
                        dst[_ds(i, 64), cols] = pltpu.bitcast(src[_ds(i, 128), cols], I32)
                        return carry

                    lax.fori_loop(0, NG, body, 0)

        U = BL[tr + 1] - BL[tr]
        LEN = dict(kq=8 * TICKS, v=4 * TICKS, s=80, o=0, m=8)
        order = [("kq", 0), ("s", 0)]
        for u in range(1, U - 1):
            order += [("kq", u), ("v", u - 1), ("s", u), ("o", u - 1), ("m", u - 1)]
        order += [("kq", U - 1), ("s", U - 1), ("v", U - 2), ("v", U - 1), ("o", U - 2), ("o", U - 1),
                  ("m", U - 2), ("m", U - 1)]
        pace = _Pacer(z)
        lane_head = lax.broadcasted_iota(I32, (128, 128), 1) // DH
        row_head = lax.broadcasted_iota(I32, (128, 128), 0) // DH

        def group(u):
            g = BL[tr] + u
            cols = _ds(g, 128)
            ks, pks, qms, pqs, vts, ss, pp, fs, ams = abufs[u % 2]
            st = {}

            def proj(i, w):
                y = _nn(pace.lhs(xna[_blk(i, 64), :]), _up(wa[w][:, cols]) if CFG["WW"] else (wk, wq, wv)[w][:, cols])
                pace.done(y)
                return y

            def proj_k(i):
                k = proj(i, 0)
                pk = _phi(k)
                ks[z, _blk(i, 64), :], pks[z, _blk(i, 64), :] = _pk2(k, pk)
                ps = _fold8(pk, jnp.add)
                st["pksum"] = ps if i == 0 else st["pksum"] + ps

            def proj_q(j):
                q = proj(j, 1)
                qj, pq = _pk2(q * QSCALE, _phi(q))
                for i in range(4):
                    for c in range(4):
                        qms[j][z, i, _blk(c, 16), :] = jnp.where(lane_head[:16] == c ^ i, qj[_blk(i, 16)], 0)
                pqs[z, _blk(j, 64), :] = _skew_rows(pq)

            def proj_v(i):
                vts[z, :, _blk(i)] = vt = pltpu.bitcast(proj(i, 2).astype(BF16).T, I32)
                deadline(pace.now + CFG["VK"], vt[56:])

            def deadline(tick, x):
                if tick < U * sum(LEN.values()):
                    pace.sink(tick, x)

            def qk(j, i):
                n = j * 128 + (i + 1) * DH
                s = _nt((pace.lhs if i == 3 else _up)(ks[0, 0:n // 2, :]), _up(qms[j][0, i]))
                sd = s[n - DH:] + cmask[...]
                s = jnp.concatenate([s[:n - DH], sd], axis=0) if n > DH else sd
                ss[j][z, i, 16:16 + n, :] = s
                m = jnp.max(_fold8(s, jnp.maximum), axis=0, keepdims=True)
                ss[j][z, i, 0:8, :] = st['m', j] = jnp.broadcast_to(m, (8, 128))

            def ex(plan):
                EC = CFG["EC"]
                zt = pltpu.bitcast(pace.zero(st['m', js[CFG['GJ']]]), F32)
                for j in js:
                    n = (j + 1) * 128
                    l = [None] * 4
                    for r in range(0, n, EC):
                        tick, gated = next(plan)
                        zt = (yield)[1] if gated else zt
                        if r == 0:
                            m = [ss[j][0, i, 0:8, :] for i in range(4)]
                        ps = []
                        for i in range(4):
                            if r < j * 128 + (i + 1) * DH:
                                m[i] = m[i] + zt if gated or r == 0 else m[i]
                                p = jnp.exp2(ss[j][0, i, 16 + r:16 + r + EC, :] - jnp.concatenate([m[i]] * (EC // 8)))
                                l[i] = _fold8(p, jnp.add) if r == 0 else l[i] + _fold8(p, jnp.add)
                                ps.append(p)
                        ps = _skew([jnp.zeros((EC // 2, 128), I32)] * (4 - len(ps)) + _tiles(_pk(jnp.concatenate(ps, axis=1))))
                        pp[j][z, r // 2:(r + EC) // 2, :] = jnp.concatenate(ps, axis=1)
                        deadline(tick + CFG["D2"], (ps[0] | ps[1] | ps[2] | ps[3])[:8] if CFG["ALL"] else ps[3][:8])
                        deadline(tick, (l[0] + l[1]) + (l[2] + l[3]))
                    row = lax.broadcasted_iota(I32, (8, 128), 0)
                    tot = jnp.ones((8, 128), F32)
                    for h, v in enumerate(_skew(l)):
                        tot = jnp.where(row == h, jnp.sum(v, axis=0, keepdims=True), tot)
                    fs[z, j] = f = (1.0 - gate[g]) / tot
                    deadline(tick + CFG["FK"], f)

            def mem():
                zm = jnp.where(lax.broadcasted_iota(I32, (16, 128), 0) == lane_head[:16],
                               jnp.broadcast_to(zs[g], (16, 128)), 0.0)
                r = _nt(jnp.concatenate([zm, mt[g]], axis=0).astype(BF16), _up(pqs[0]))
                f = jnp.concatenate([gate[g]] * 4, axis=1) / (r[0:8] + 1e-6)
                for h in range(4):
                    ams[z, _blk(h, DH), :] = r[16 + h * DH:16 + (h + 1) * DH] * f[h:h + 1]

            def pv(j):
                n = (j + 1) * 128
                outs = []
                for h in range(4):
                    o = _nn(_up(vts[0, _blk(h, DH // 2), 0:n]), _up(pp[j][0, :, _blk(h)]))
                    f = fs[0, j, h:h + 1, :]
                    outs.append(o * f + ams[0, _blk(h, DH), _blk(j)])
                o = pltpu.bitcast(jnp.concatenate(outs, axis=0).astype(BF16).T, I32)
                obuf[_blk(j, 64), cols] = o = _skew_rows(o)
                deadline(pace.now + (CFG['OK'] if u < U - 2 else 0 if u == U - 2 else CFG['OL']) + 2 * j, functools.reduce(jnp.bitwise_or, [o[_blk(c, 8)] for c in range(8)]))

            def upd():
                mt[g] = new = mt[g] + jnp.where(lane_head == row_head, _nn(pace.lhs(vts[0]), _up(pks[0])), 0.0)
                deadline(pace.now + CFG['OK'], _fold8(new, jnp.add))
                zs[g] = zs[g] + jnp.sum(st["pksum"], axis=0, keepdims=True)

            js = CFG["JS"]

            def st_kq():
                for i in range(4):
                    proj_k(i)
                for j in js:
                    proj_q(j)

            def st_v():
                for i in range(4):
                    proj_v(i)

            def st_s():
                for j in js:
                    for i in (CFG['J0'] if j == 0 else (3, 2, 1, 0)):
                        qk(j, i)
                n = 10 * 128 // CFG["EC"]
                i0 = order.index(("s", u)) + 1
                i1 = order.index(("s", u + 1)) + 1 if u + 1 < U else len(order) - 2
                slots, starts, t = [], [], pace.now
                for name, _ in order[i0:i1]:
                    slots += [t + d for d in range(LEN[name]) for _ in range(CFG["WT"][name])]
                    if name in ("kq", "v"):
                        starts += list(range(t, t + LEN[name], TICKS))
                    t += LEN[name]
                slots = slots[:len(slots) - CFG['CUT']]
                plan, points = [], []
                for c in range(n):
                    tick = slots[c * len(slots) // n]
                    cand = [p + v for p in starts for v in (0, TICKS - 1)
                            if p + (TICKS + v) // 2 + 7 + CFG["EK"] <= tick]
                    gated = bool(cand) and cand[-1] not in points
                    plan.append((tick, gated))
                    if gated:
                        points.append(cand[-1])
                pace.at(points, ex(iter(plan)))

            def st_o():
                mem()
                for j in js:
                    pv(j)

            return dict(kq=st_kq, v=st_v, s=st_s, o=st_o, m=upd)

        gs = [group(u) for u in range(U)]
        for name, u in order:
            gs[u][name]()
        assert not pace.sinks and not pace.side

    with jax.named_scope("aloop"):
        for tr in range(NCH):
            a_trip(tr)

    def _prepare_b():
        def permute(words, dst, i, hp):
            for half in range(2):
                ev, od = (words[_blk(2 * n + half, 8)] for n in range(2))
                dst[i, pl.ds(32 * half + hp, NG, stride=PST), :] = (ev & 0xFFFF) | (od << 16)
                dst[i, pl.ds(32 * half + 16 + hp, NG, stride=PST), :] = (
                    lax.shift_right_logical(ev, 16) | (od & -0x10000))

        with jax.named_scope('latewait'):
            for c in late:
                c.wait()

        row = lax.broadcasted_iota(I32, (128, 128), 0)
        src_col = (row // 64 * 2 + row % 2) * DH + (row // 32 % 2 * 8 + row // 2 % 8) * 2 + row // 16 % 2
        mover = jnp.where(lax.broadcasted_iota(I32, (128, 128), 1) == src_col, 1.0, 0.0).astype(BF16)
        for i in range(NG):
            words = pltpu.bitcast(wqkv[_blk(i), 0:2 * D].T, I32)
            for hp in range(H // 2):
                for part in range(2):
                    permute(words[_blk(part * (H // 2) + hp, 32)], wb[part], i, hp)
                zt = jnp.concatenate([words[_blk(8 * hp, 8)] & z] * 4)
                permute(pltpu.bitcast(wob[_blk(hp, 64), _blk(i)], I32) | zt, wb[3], i, hp)
                rows, cols = 4 * i + hp // 4, _blk(hp % 4, 256)
                wa[3][_blk(rows, 16), cols] = (pltpu.bitcast(wo[_blk(rows, 32), cols], I32)
                                               | jnp.concatenate([zt[:16]] * 2, axis=1))
        for c in range(NG):
            for i0 in range(0, NG, 4):
                words = _pk(_nt(mover, wqkv[i0 * 128:(i0 + 4) * 128, _blk(2 * NG + c)]))
                for i, tile in enumerate(_tiles(words)):
                    for n in range(8):
                        wb[2][i0 + i, pl.ds(n % 4 * 16 + 2 * c + n // 4, NG, stride=PST), :] = tile[_blk(n, 8)]

    with jax.named_scope("prep"):
        pl.when(it == 0)(_prepare_b)

    NR = L // (NB * RB)

    def out_copy(seg, tr):
        return pltpu.make_async_copy(xout.at[_ds(tr, NB * RB)], out_ref.at[_ds(seg * NR + tr, NB * RB)],
                                     sems.at[3 * NCH + 5 + tr])

    def r_trip(tr, carry):
        pl.when(it > NSEG)(out_copy(jnp.maximum(seg - 1, 0), tr).wait)
        pace = _Pacer(z)

        def a_out(i, t):
            y = _nn(pace.lhs(obuf[_ds(tr * NB + i, RB // 2), :]), _up(wa[3][:, _blk(t)]))
            xm[i][last(t == NG - 1), :, _blk(t)] = xcur[_ds(tr * NB + i, RB), _blk(t)] + y
            return y

        def b_proj(i, part, t):
            y = _nt(pace.lhs(xnb[i][0]), _up(jnp.concatenate(
                [wb[part][k, pl.ds(t * PST, 64), :] for k in range(NG)], axis=1)))
            if part == 0:
                qk_[i][z, t, KR:KR + RB, :] = y * QSCALE
            else:
                buf = (qk_, vo)[part - 1]
                buf[i][last(t == NG - 1), t, HALO:KR, :] = y
                if i + 1 < NB:
                    buf[i + 1][z, t, 0:HALO, :] = y[RB - HALO:]
            return y

        def b_out(i, t):
            x = xm[i][0, :, _blk(t)] + _nn(pace.lhs(ob2[i][0]), _up(jnp.concatenate(
                [wb[3][t, pl.ds(k * PST, 64), :] for k in range(NG)], axis=0)))
            xres[seg, _ds(tr * NB + i, RB), _blk(t)] = x
            xout[_ds(tr * NB + i, RB), _blk(t)] = x.astype(BF16)
            return x

        def mid_ln(i):
            for r in range(RB // 16):
                now, zt = yield
                y = _layernorm(lambda p: xm[i][zz[p] if p else 0, _blk(r, 16), :], jnp.concatenate([zt, zt]))
                xnb[i][last(r == RB // 16 - 1), _blk(r, 8), :] = y
                pace.sink(now + CFG["LNK"], y[:, D - 128:])

        def next_ln():
            n = NB * RB // 16
            for r in range(n):
                now, zt = yield
                rows = _ds(tr * n + r, 16)

                def load(p):
                    if p:
                        return stage[r % 3][zz[p]]
                    x = xin[_ds(nseg * (L // 16) + tr * n + r, 16), :].astype(F32)
                    x = jnp.where(it < NSEG - 1, x, xres[nseg, rows, :])
                    stage[r % 3][z] = x
                    xcur[rows, :] = x
                    return x

                y = _layernorm(load, jnp.concatenate([zt, zt]))
                xna[_ds(tr * n + r, 8), :] = y
                pace.sink(now + CFG["LNK"], y[:, D - 128:])

        def b_prob(i):
            for r in range(0, RB, 8):
                lg = []
                for w in range(W):
                    if w % CFG["NW"] == 0:
                        now, zt = yield
                    if w == 0:
                        q = [qk_[i][0, t, KR + r:KR + r + 8, :] for t in range(NG)]
                    a = zt
                    for t in range(NG):
                        a = a + q[t] * qk_[i][0, t, pl.ds(r + HALO - DIL * w, 8), :]
                    a = a + pltpu.roll(a, 64, 1)
                    a = a + pltpu.roll(a, 32, 1)
                    if i * RB + r < DIL * w:
                        pos = seg * L + tr * (NB * RB) + r + lax.broadcasted_iota(I32, (8, 128), 0)
                        a = jnp.where(pos >= DIL * w, a, NEG)
                    lg.append(a)
                m = functools.reduce(jnp.maximum, lg)
                e = [jnp.exp2(a - m) for a in lg]
                tot = functools.reduce(jnp.add, e)
                if CFG["DEF"]:
                    for w, p in enumerate(e + [tot]):
                        pb[i][last(r == RB - 8), w, r:r + 8, :] = p
                else:
                    inv = 1.0 / tot
                    for w in range(W):
                        pb[i][z, w, r:r + 8, :] = p = e[w] * inv
                pace.sink(now + CFG["PK"], p)

        def b_mix(i):
            now, _ = yield
            for r in range(RB // 16):
                p = [pb[i][0, w, _blk(r, 16), :] for w in range(W)]
                if CFG["DEF"]:
                    inv = 1.0 / pb[i][0, W, _blk(r, 16), :]
                for t in range(NG):
                    o = None
                    for c in range(4):
                        vv = vo[i][0, t, pl.ds(r * 16 + HALO - DIL * c - 8, 24), :]
                        for w, vw in ((c, vv[8:]), (c + 4, vv[:16])):
                            o = p[w] * vw if o is None else o + p[w] * vw
                    ob2[i][last(r * NG + t == RB // 2 - 1), _blk(r, 8), _blk(t)] = o = _pk(o * inv if CFG["DEF"] else o)
                    pace.sink(now + CFG["MK"] + (r * NG + t) * CFG["MS"] // 4, o)

        def carry_halo():
            for buf in (qk_, vo):
                _, zt = yield
                buf[0][z, :, 0:HALO, :] = buf[NB - 1][0, :, RB:KR, :] + jnp.concatenate([zt, zt])

        pace.at([TICKS * ((5 * NB - 1) * NG + n) for n in (5, 6)], carry_halo())
        pt = functools.partial
        mxu = [pt(a_out, i, t) for i in range(NB) for t in range(NG)]
        mxu += [pt(b_proj, i, part, t) for i in range(NB) for part in range(2) for t in range(NG)]
        mxu += [pt(b_proj, i, 2, t) for i in range(NB) for t in range(NG)]
        mxu += [pt(b_out, i, t) for i in range(NB) for t in range(NG)]
        V = TICKS
        for i in range(NB):
            pace.at([V * (i + 1) * NG - 1 + n * CFG["LS"] for n in range(RB // 16)], mid_ln(i))
            s0 = V * (NB * NG + (i + 1) * 2 * NG)
            pace.at([s0 + n * CFG["PS"][i] // 2 for n in range(V * W // CFG["NW"])], b_prob(i))
            pace.at([V * (3 * NB * NG + (i + 1) * NG) - 1], b_mix(i))
        n1 = CFG["N1"]
        pace.at([V * NB * NG + CFG["N0"] + n * CFG["NS"] for n in range(n1)]
                + [V * (5 * NB - 1) * NG + n * CFG["LS"] - 1 for n in range(NB * RB // 16 - n1)], next_ln())
        for f in mxu:
            pace.done(f())
        assert not pace.sinks and not pace.side
        pl.when(it >= NSEG)(out_copy(seg, tr).start)
        return carry

    with jax.named_scope("rloop"):
        lax.fori_loop(0, NR, r_trip, 0)

    @pl.when(it == 2 * NSEG - 1)
    def _finish():
        for tr in range(NR):
            out_copy(seg, tr).wait()


@jax.jit
def pallas_interleave_layers__memory_aug_infini_attn__sliding_local_dilated__prompt_kernel(A_x, A_wq, A_wk, A_wv, A_wo, A_beta, B_x, B_wqkv, B_wo):
    del B_x
    any_spec = pl.BlockSpec(memory_space=pl.ANY)
    vmem = pltpu.VMEM
    NB = CFG["NB"]
    group_bufs = [
        vmem((1, L // 2, 128), I32),
        vmem((1, L // 2, 128), I32),
        [vmem((1, 4, 64, 128), I32)] * 4,
        vmem((1, L // 2, 128), I32),
        vmem((1, 64, L), I32),
        [vmem((1, 4, 128 * (j + 1) + 24, 128), F32) for j in range(4)],
        [vmem((1, 64 * (j + 1), 512), I32) for j in range(4)],
        vmem((1, 4, 8, 128), F32),
        vmem((1, 128, L), F32),
    ]
    out = pl.pallas_call(
        _kernel,
        grid=(2 * NSEG,),
        in_specs=[any_spec] * 8,
        out_specs=any_spec,
        out_shape=jax.ShapeDtypeStruct((S, D), A_x.dtype),
        scratch_shapes=[
            vmem((S, D), BF16),
            vmem((D, D), BF16),
            vmem((D, D), BF16),
            vmem((D, D), BF16),
            vmem((D, D), BF16),
            vmem((D, 3 * D), BF16),
            vmem((D, D), BF16),
            vmem((H,), BF16),
            [vmem((D // 2, D), I32)] * 4,
            [vmem((NG, NG * PST, 128), I32)] * 4,
            pltpu.SemaphoreType.DMA((3 * (len(CFG['BL']) - 1) + 8,)),
            vmem((NSEG, L, D), F32),
            vmem((L, D), F32),
            [vmem((1, 16, D), F32)] * 3,
            vmem((L, D), BF16),
            vmem((L // 2, D), I32),
            vmem((L // 2, D), I32),
            vmem((NG, 8, 128), F32),
            vmem((DH, 128), F32),
            vmem((NG, 128, 128), F32),
            vmem((NG, 1, 128), F32),
            [group_bufs] * 2,
            [vmem((1, RB, D), F32)] * NB,
            [vmem((1, RB // 2, D), I32)] * NB,
            [vmem((1, RB // 2, D), I32)] * NB,
            [vmem((1, NG, KR + RB + CFG.get("P1", 0), 128), F32)] * NB,
            [vmem((1, NG, KR + CFG.get("P2", 0), 128), F32)] * NB,
            [vmem((1, W + 1, RB + CFG.get('P3', 0), 128), F32)] * NB,
        ],
        compiler_params=pltpu.CompilerParams(
            dimension_semantics=("arbitrary",), vmem_limit_bytes=110 * 1024 * 1024),
        name="fused_layers",
    )(A_x.reshape(S, D), A_wq, A_wk, A_wv, A_wo, A_beta, B_wqkv, B_wo)
    return out.reshape(A_x.shape)
```

```python
import functools

import jax
import jax.numpy as jnp
from jax import lax
import jax.experimental.pallas as pl
import jax.experimental.pallas.tpu as pltpu

F32 = jnp.float32
BF16 = jnp.bfloat16
I32 = jnp.int32

S, D, H, DH = 2048, 1024, 32, 32
NSEG, L = 4, 512
W, DIL = 8, 2
QSCALE = DH ** -0.5 * 1.4426950408889634
NEG = -1e30

NG = D // 128
A_SPLIT = (0, 2, 8)
RB, NB = 128, 2
NR = L // (NB * RB)
HALO = 16
KR = HALO + RB
PST = 68
TICKS = 16
QK_TICKS = (3, 12, 18, 32)


def _nn(a, b):
    return jnp.dot(a, b, preferred_element_type=F32)


def _nt(a, b):
    return lax.dot_general(a, b, (((1,), (1,)), ((), ())), preferred_element_type=F32)


def _pack(x):
    return pltpu.bitcast(x.astype(BF16), I32)


def _pack_tiles(xs):
    return _tiles(_pack(jnp.concatenate(xs, axis=1)))


def _bf16(words):
    return pltpu.bitcast(words, BF16)


def _blk(i, n=128):
    return slice(i * n, (i + 1) * n)


def _ds(i, n):
    return pl.ds(i * n if isinstance(i, int) else pl.multiple_of(i * n, n), n)


def _tiles(x):
    return [x[:, _blk(t)] for t in range(x.shape[1] // 128)]


def _fold8(x, op):
    return functools.reduce(op, [x[r:r + 8] for r in range(0, x.shape[0], 8)])


def _phi(t):
    return jnp.where(t > 0, t + 1.0, jnp.exp(t))


def _skew(xs):
    quarter = lax.broadcasted_iota(I32, xs[0].shape, 1) // DH
    for bit in (1, 2):
        xs = [jnp.where((quarter & bit) != 0, xs[i ^ bit], xs[i]) for i in range(4)]
    return xs


def _skew_rows(x):
    n = x.shape[0] // 4
    return jnp.concatenate(_skew([x[_blk(i, n)] for i in range(4)]), axis=0)


def _layernorm(load, zero=None):
    tiles = _tiles(load(0))
    s = functools.reduce(jnp.add, tiles if zero is None else [zero] + tiles)
    m = jnp.sum(s, axis=-1, keepdims=True) * (1.0 / D)
    s = functools.reduce(jnp.add, [(x - m) * (x - m) for x in _tiles(load(1))])
    rs = lax.rsqrt(jnp.sum(s, axis=-1, keepdims=True) * (1.0 / D) + 1e-5)
    return _pack((load(2) - m) * rs)


class _Pacer:
    def __init__(self, z, total):
        self.z, self.total, self.now, self.due, self.waiting = z, total, 0, {}, {}

    def zero(self, x):
        return (x if x.dtype == I32 else pltpu.bitcast(x, I32)) & self.z

    def deadline(self, tick, x):
        assert tick >= self.now
        if tick < self.total:
            zt = self.zero(x)
            self.due[tick] = self.due[tick] | zt if tick in self.due else zt

    def lhs(self, words, ticks=None):
        cols = _tiles(words)
        n = words.shape[0] // 8
        for c in range(0, len(cols), 4):
            zts = [self.due.pop(self.now + r, None) for r in range(ticks or n)]
            self.now += len(zts)
            if any(zt is not None for zt in zts):
                rows = [cols[c][_blk(r, 8)] for r in range(n)]
                zts += [None] * (n - len(zts))
                cols[c] = jnp.concatenate([v if zt is None else v | zt for v, zt in zip(rows, zts)])
        return _bf16(jnp.concatenate(cols, axis=1))

    @staticmethod
    def ready(start, v):
        return start + (TICKS + v) // 2 + 7

    def at(self, points, gen):
        next(gen, None)
        for p in points:
            self.waiting.setdefault(p, []).append(gen)

    def done(self, y):
        start = self.now - TICKS
        for v in range(TICKS):
            for gen in self.waiting.pop(start + v, []):
                try:
                    gen.send((self.ready(start, v), pltpu.bitcast(self.zero(y[_blk(v, 8)]), F32)))
                except StopIteration:
                    pass

    def close(self):
        assert self.now == self.total and not self.due and not self.waiting


def _kernel(x_hbm, wq_hbm, wk_hbm, wv_hbm, wo_hbm, beta_hbm, wqkv_hbm, wob_hbm, out_hbm,
            xin, wq, wk, wv, wo, wqkv, wob, beta, wa, wb, sems,
            xres, xcur, stage, xout, xna, oa, gate, cmask, mem_m, mem_z, group_bufs,
            xmid, xnb, ob, kq_buf, v_buf, p_buf):
    it = pl.program_id(0)
    seg = it % NSEG
    nseg = (it + 1) % NSEG
    zz = [it // (2 * NSEG << n) for n in range(3)]
    z = zz[0]
    batches = len(A_SPLIT) - 1

    def a_copies(b):
        cols = pl.ds(A_SPLIT[b] * 128, (A_SPLIT[b + 1] - A_SPLIT[b]) * 128)
        return [pltpu.make_async_copy(src.at[:, cols], dst.at[:, cols], sems.at[3 * b + i])
                for i, (src, dst) in enumerate(((wk_hbm, wk), (wq_hbm, wq), (wv_hbm, wv)))]

    def late_copies():
        pairs = ((wqkv_hbm, wqkv), (wob_hbm, wob), (wo_hbm, wo), (x_hbm.at[L:S], xin.at[L:S]))
        return [pltpu.make_async_copy(src, dst, sems.at[3 * batches + i])
                for i, (src, dst) in enumerate(pairs)]

    def out_copy(s, tr):
        return pltpu.make_async_copy(xout.at[_ds(tr, NB * RB)], out_hbm.at[_ds(s * NR + tr, NB * RB)],
                                     sems.at[3 * batches + 6 + tr])

    @pl.when(it == 0)
    def _start():
        beta_copy = pltpu.make_async_copy(beta_hbm, beta, sems.at[3 * batches + 4])
        x_copy = pltpu.make_async_copy(x_hbm.at[0:L], xin.at[0:L], sems.at[3 * batches + 5])
        for c in [beta_copy, x_copy] + a_copies(0):
            c.start()

        def clear(i, carry):
            xres[1:, _ds(i, 32), :] = jnp.zeros((NSEG - 1, 32, D), F32)
            return carry

        lax.fori_loop(0, L // 32, clear, 0)
        beta_copy.wait()
        g = jax.nn.sigmoid(beta[...].astype(F32).reshape(1, H))
        eye = lax.broadcasted_iota(I32, (H, H), 0) == lax.broadcasted_iota(I32, (H, H), 1)
        g = jnp.sum(jnp.where(eye, jnp.broadcast_to(g, (H, H)), 0.0), axis=1, keepdims=True)
        g = jnp.broadcast_to(g, (H, 128))
        for i in range(NG):
            gate[i] = jnp.concatenate([g[_blk(i, 4)]] * 2)
        cmask[...] = jnp.where(lax.broadcasted_iota(I32, (DH, 128), 0)
                               <= lax.broadcasted_iota(I32, (DH, 128), 1) % DH, 0.0, NEG)
        x_copy.wait()

        def first_ln(i, carry):
            x = xin[_ds(i, RB), :].astype(F32)
            xcur[_ds(i, RB), :] = x
            xna[_ds(i, RB // 2), :] = _layernorm(lambda p: xcur[_ds(i + zz[p], RB), :] if p else x)
            return carry

        lax.fori_loop(0, L // RB, first_ln, 0)

    @pl.when(seg == 0)
    def _reset():
        mem_m[...] = jnp.zeros(mem_m.shape, F32)
        mem_z[...] = jnp.zeros(mem_z.shape, F32)
        kq_buf[0][0, :, 0:HALO, :] = jnp.zeros((NG, HALO, 128), F32)
        v_buf[0][0, :, 0:HALO, :] = jnp.zeros((NG, HALO, 128), F32)

    def a_batch(b):
        first, end = A_SPLIT[b], A_SPLIT[b + 1]

        @pl.when(it == 0)
        def _weights():
            cols = slice(first * 128, end * 128)
            for n, (c, src) in enumerate(zip(a_copies(b), (wk, wq, wv))):
                c.wait()
                if n == 2:
                    for nxt in a_copies(b + 1) if b + 1 < batches else late_copies():
                        nxt.start()

                def to_words(i, carry, src=src, dst=wa[n]):
                    dst[_ds(i, 64), cols] = pltpu.bitcast(src[_ds(i, 128), cols], I32)
                    return carry

                lax.fori_loop(0, NG, to_words, 0)

        order = [("kq", first), ("scores", first)]
        for g in range(first + 1, end - 1):
            order += [("kq", g), ("v", g - 1), ("scores", g), ("out", g - 1), ("update", g - 1)]
        order += [("kq", end - 1), ("scores", end - 1)]
        order += [(name, g) for name in ("v", "out", "update") for g in (end - 2, end - 1)]
        order = [(name, g) for name, g in order if name != "update" or g < NG - 2]
        ticks = dict(kq=8 * TICKS, v=4 * TICKS, scores=sum(QK_TICKS), out=8, update=8)
        pace = _Pacer(z, sum(ticks[name] for name, _ in order))
        lane_head = lax.broadcasted_iota(I32, (128, 128), 1) // DH
        row_head = lax.broadcasted_iota(I32, (128, 128), 0) // DH

        def group(g):
            ks, pks, qs, pqs, vts, ss, ps, fs, ms = group_bufs[g % 2]
            st = {}

            def proj(i, w):
                y = _nn(pace.lhs(xna[_blk(i, 64), :]), _bf16(wa[w][:, _blk(g)]))
                pace.done(y)
                return y

            def proj_kq():
                for i in range(4):
                    k = proj(i, 0)
                    pk = _phi(k)
                    ks[z, _blk(i, 64), :], pks[g // 2 + z, _blk(i, 64), :] = _pack_tiles([k, pk])
                    st["z"] = st["z"] + _fold8(pk, jnp.add) if i else _fold8(pk, jnp.add)
                for j in range(4):
                    q = proj(j, 1)
                    q, pq = _pack_tiles([q * QSCALE, _phi(q)])
                    for i in range(4):
                        for c in range(4):
                            qs[j][z, i, _blk(c, 16), :] = jnp.where(lane_head[:16] == c ^ i, q[_blk(i, 16)], 0)
                    pqs[z, _blk(j, 64), :] = _skew_rows(pq)

            def proj_v():
                for i in range(4):
                    vts[g // 2 + z, :, _blk(i)] = vt = pltpu.bitcast(proj(i, 2).astype(BF16).T, I32)
                    pace.deadline(pace.now + 20, vt[56:])

            def softmax(plan):
                zt = pltpu.bitcast(pace.zero(st["max", 1]), F32)
                for j in range(4):
                    l = [None] * 4
                    for r in range(0, (j + 1) * 128, 16):
                        tick, wait = next(plan)
                        zt = (yield)[1] if wait else zt
                        if r == 0:
                            m = [ss[j][0, i, 0:8, :] for i in range(4)]
                        es = []
                        for i in range(4):
                            if r < j * 128 + (i + 1) * DH:
                                m[i] = m[i] + zt if wait or r == 0 else m[i]
                                e = jnp.exp2(ss[j][0, i, 16 + r:32 + r, :] - jnp.concatenate([m[i]] * 2))
                                l[i] = l[i] + _fold8(e, jnp.add) if r else _fold8(e, jnp.add)
                                es.append(e)
                        es = _skew([jnp.zeros((8, 128), I32)] * (4 - len(es)) + _pack_tiles(es))
                        ps[j][z, r // 2:r // 2 + 8, :] = jnp.concatenate(es, axis=1)
                        pace.deadline(tick + 1, es[3])
                        pace.deadline(tick, (l[0] + l[1]) + (l[2] + l[3]))
                    total = jnp.ones((8, 128), F32)
                    for h, v in enumerate(_skew(l)):
                        total = jnp.where(lax.broadcasted_iota(I32, (8, 128), 0) == h,
                                          jnp.sum(v, axis=0, keepdims=True), total)
                    fs[z, j] = f = (1.0 - gate[g]) / total
                    pace.deadline(tick + 6, f)

            def scores():
                for j in range(4):
                    for i in (3, 2, 1, 0):
                        n = j * 128 + (i + 1) * DH
                        k = ks[0, 0:n // 2, :]
                        s = _nt(pace.lhs(k, QK_TICKS[j]) if i == 3 else _bf16(k), _bf16(qs[j][0, i]))
                        diag = s[n - DH:] + cmask[...]
                        s = jnp.concatenate([s[:n - DH], diag], axis=0) if n > DH else diag
                        ss[j][z, i, 16:16 + n, :] = s
                        m = jnp.max(_fold8(s, jnp.maximum), axis=0, keepdims=True)
                        ss[j][z, i, 0:8, :] = st["max", j] = jnp.broadcast_to(m, (8, 128))
                stop = order.index(("scores", g + 1)) + 1 if g + 1 < end else order.index(("out", g))
                slots, starts, t = [], [], pace.now
                for name, _ in order[order.index(("scores", g)) + 1:stop]:
                    if name in ("kq", "v", "scores"):
                        slots += range(t, t + ticks[name])
                    if name in ("kq", "v"):
                        starts += range(t, t + ticks[name], TICKS)
                    t += ticks[name]
                plan, points, pieces = [], [], 10 * 128 // 16
                for c in range(pieces):
                    tick = slots[c * (len(slots) - 2) // pieces]
                    early = [p + v for p in starts for v in (0, TICKS - 1) if pace.ready(p, v) + 8 <= tick]
                    plan.append((tick, bool(early) and early[-1] not in points))
                    if plan[-1][1]:
                        points.append(early[-1])
                pace.at(points, softmax(iter(plan)))

            def out():
                zrows = jnp.where(lax.broadcasted_iota(I32, (16, 128), 0) == lane_head[:16],
                                  jnp.broadcast_to(mem_z[g], (16, 128)), 0.0)
                r = _nt(jnp.concatenate([zrows, mem_m[g]], axis=0).astype(BF16), _bf16(pqs[0]))
                mem_z[g] = mem_z[g] + jnp.sum(st["z"], axis=0, keepdims=True)
                f = jnp.concatenate([gate[g]] * 4, axis=1) / (r[0:8] + 1e-6)
                for h in range(4):
                    ms[z, _blk(h, DH), :] = r[16 + h * DH:16 + (h + 1) * DH] * f[h:h + 1]
                for j in range(4):
                    heads = []
                    for h in range(4):
                        vt = vts[g // 2, _blk(h, DH // 2), 0:(j + 1) * 128]
                        o = _nn(pace.lhs(vt) if h == 3 else _bf16(vt), _bf16(ps[j][0, :, _blk(h)]))
                        heads.append(o * fs[0, j, h:h + 1, :] + ms[0, _blk(h, DH), _blk(j)])
                    o = pltpu.bitcast(jnp.concatenate(heads, axis=0).astype(BF16).T, I32)
                    oa[_blk(j, 64), _blk(g)] = o = _skew_rows(o)
                    slack = 28 if g < end - 2 else (12, 10, 9, 7)[j] if g == end - 2 else 18
                    pace.deadline(pace.now + slack, _fold8(o, jnp.bitwise_or))

            def update():
                lag = (g >= NG - 2 - 2 * seg).astype(I32)
                new = _nn(pace.lhs(vts[g // 2 + lag]), _bf16(pks[g // 2 + lag]))
                mem_m[g + 2 * lag] = new = mem_m[g + 2 * lag] + jnp.where(lane_head == row_head, new, 0.0)
                pace.deadline(pace.now + 28, _fold8(new, jnp.add))

            return dict(kq=proj_kq, v=proj_v, scores=scores, out=out, update=update)

        groups = {g: group(g) for g in range(first, end)}
        for name, g in order:
            groups[g][name]()
        pace.close()

    for b in range(batches):
        a_batch(b)

    @pl.when(it == 0)
    def _reorder_b_weights():
        def move(words, dst, i, pair):
            for a in range(2):
                even, odd = (words[_blk(2 * n + a, 8)] for n in range(2))
                dst[i, pl.ds(32 * a + pair, NG, stride=PST), :] = (even & 0xFFFF) | (odd << 16)
                dst[i, pl.ds(32 * a + 16 + pair, NG, stride=PST), :] = (
                    lax.shift_right_logical(even, 16) | (odd & -0x10000))

        for c in late_copies():
            c.wait()
        row = lax.broadcasted_iota(I32, (128, 128), 0)
        col = (row // 64 * 2 + row % 2) * DH + (row // 32 % 2 * 8 + row // 2 % 8) * 2 + row // 16 % 2
        mover = jnp.where(lax.broadcasted_iota(I32, (128, 128), 1) == col, 1.0, 0.0).astype(BF16)
        for i in range(NG):
            words = pltpu.bitcast(wqkv[_blk(i), 0:2 * D].T, I32)
            for pair in range(H // 2):
                for part in range(2):
                    move(words[_blk(part * (H // 2) + pair, 32)], wb[part], i, pair)
                zt = jnp.concatenate([words[_blk(8 * pair, 8)] & z] * 4)
                move(pltpu.bitcast(wob[_blk(pair, 64), _blk(i)], I32) | zt, wb[3], i, pair)
                rows, cols = 4 * i + pair // 4, _blk(pair % 4, 256)
                wa[3][_blk(rows, 16), cols] = (pltpu.bitcast(wo[_blk(rows, 32), cols], I32)
                                               | jnp.concatenate([zt[:16]] * 2, axis=1))
        for c in range(NG):
            for i0 in range(0, NG, 4):
                words = _pack(_nt(mover, wqkv[i0 * 128:(i0 + 4) * 128, _blk(2 * NG + c)]))
                for i, tile in enumerate(_tiles(words)):
                    for n in range(8):
                        wb[2][i0 + i, pl.ds(n % 4 * 16 + 2 * c + n // 4, NG, stride=PST), :] = tile[_blk(n, 8)]

    def row_trip(tr, carry):
        @pl.when(it > NSEG)
        def _sent():
            out_copy(jnp.maximum(seg - 1, 0), tr).wait()

        pace = _Pacer(z, 5 * NB * NG * TICKS)

        def a_out(i, t):
            y = _nn(pace.lhs(oa[_ds(tr * NB + i, RB // 2), :]), _bf16(wa[3][:, _blk(t)]))
            xmid[i][z, :, _blk(t)] = xcur[_ds(tr * NB + i, RB), _blk(t)] + y
            return y

        def b_proj(i, part, t):
            y = _nt(pace.lhs(xnb[i][0]), _bf16(jnp.concatenate(
                [wb[part][k, pl.ds(t * PST, 64), :] for k in range(NG)], axis=1)))
            if part == 0:
                kq_buf[i][z, t, KR:KR + RB, :] = y * QSCALE
            else:
                buf = (kq_buf, v_buf)[part - 1]
                buf[i][z, t, HALO:KR, :] = y
                if i + 1 < NB:
                    buf[i + 1][z, t, 0:HALO, :] = y[RB - HALO:]
            return y

        def b_out(i, t):
            x = xmid[i][0, :, _blk(t)] + _nn(pace.lhs(ob[i][0]), _bf16(jnp.concatenate(
                [wb[3][t, pl.ds(k * PST, 64), :] for k in range(NG)], axis=0)))
            xres[seg, _ds(tr * NB + i, RB), _blk(t)] = x
            xout[_ds(tr * NB + i, RB), _blk(t)] = x.astype(BF16)
            return x

        def mid_ln(i):
            for r in range(RB // 16):
                now, zt = yield
                y = _layernorm(lambda p: xmid[i][zz[p] if p else 0, _blk(r, 16), :], jnp.concatenate([zt, zt]))
                xnb[i][z, _blk(r, 8), :] = y
                pace.deadline(now + 29, y[:, D - 128:])

        def next_ln():
            n = NB * RB // 16
            for r in range(n):
                now, zt = yield
                rows = _ds(tr * n + r, 16)

                def load(p):
                    if p:
                        return stage[r % 3][zz[p]]
                    x = xin[_ds(nseg * (L // 16) + tr * n + r, 16), :].astype(F32)
                    x = jnp.where(it < NSEG - 1, x, xres[nseg, rows, :])
                    stage[r % 3][z] = x
                    xcur[rows, :] = x
                    return x

                y = _layernorm(load, jnp.concatenate([zt, zt]))
                xna[_ds(tr * n + r, 8), :] = y
                pace.deadline(now + 29, y[:, D - 128:])

        def b_softmax(i):
            for r in range(0, RB, 8):
                logits = []
                for w in range(W):
                    if w % 2 == 0:
                        now, zt = yield
                    if w == 0:
                        q = [kq_buf[i][0, t, KR + r:KR + r + 8, :] for t in range(NG)]
                    a = zt
                    for t in range(NG):
                        a = a + q[t] * kq_buf[i][0, t, pl.ds(r + HALO - DIL * w, 8), :]
                    a = a + pltpu.roll(a, 64, 1)
                    a = a + pltpu.roll(a, 32, 1)
                    if i * RB + r < DIL * w:
                        pos = seg * L + tr * (NB * RB) + r + lax.broadcasted_iota(I32, (8, 128), 0)
                        a = jnp.where(pos >= DIL * w, a, NEG)
                    logits.append(a)
                m = functools.reduce(jnp.maximum, logits)
                es = [jnp.exp2(a - m) for a in logits]
                es.append(functools.reduce(jnp.add, es))
                for w, e in enumerate(es):
                    p_buf[i][z, w, r:r + 8, :] = e
                pace.deadline(now + 28, es[W])

        def b_mix(i):
            now, _ = yield
            for r in range(RB // 16):
                es = [p_buf[i][0, w, _blk(r, 16), :] for w in range(W)]
                inv = 1.0 / p_buf[i][0, W, _blk(r, 16), :]
                for t in range(NG):
                    o = None
                    for c in range(W // 2):
                        v = v_buf[i][0, t, pl.ds(r * 16 + HALO - DIL * c - 8, 24), :]
                        for w, vw in ((c, v[8:]), (c + W // 2, v[:16])):
                            o = es[w] * vw if o is None else o + es[w] * vw
                    ob[i][z, _blk(r, 8), _blk(t)] = o = _pack(o * inv)
                    pace.deadline(now + 8 + (r * NG + t) * 7 // 4, o)

        def carry_halo():
            for buf in (kq_buf, v_buf):
                _, zt = yield
                buf[0][z, :, 0:HALO, :] = buf[NB - 1][0, :, RB:KR, :] + jnp.concatenate([zt, zt])

        span = NG * TICKS
        pace.at([(5 * NB - 1) * span + n * TICKS for n in (5, 6)], carry_halo())
        for i in range(NB):
            pace.at([(i + 1) * span - 1 + 10 * n for n in range(RB // 16)], mid_ln(i))
            pace.at([(NB + 2 * i + 2) * span + (3 - i) * n for n in range(RB // 8 * W // 2)], b_softmax(i))
            pace.at([(3 * NB + i + 1) * span - 1], b_mix(i))
        pace.at([NB * span + 88 + 10 * n for n in range(NB * RB // 16)], next_ln())
        steps = [functools.partial(a_out, i) for i in range(NB)]
        steps += [functools.partial(b_proj, i, part) for i in range(NB) for part in range(2)]
        steps += [functools.partial(b_proj, i, 2) for i in range(NB)]
        steps += [functools.partial(b_out, i) for i in range(NB)]
        for step in steps:
            for t in range(NG):
                pace.done(step(t))
        pace.close()

        @pl.when(it >= NSEG)
        def _send():
            out_copy(seg, tr).start()

        return carry

    lax.fori_loop(0, NR, row_trip, 0)

    @pl.when(it == 2 * NSEG - 1)
    def _finish():
        for tr in range(NR):
            out_copy(seg, tr).wait()


@jax.jit
def pallas_interleave_layers__memory_aug_infini_attn__sliding_local_dilated__prompt_kernel(
    A_x: jax.Array,
    A_wq: jax.Array,
    A_wk: jax.Array,
    A_wv: jax.Array,
    A_wo: jax.Array,
    A_beta: jax.Array,
    B_x: jax.Array,
    B_wqkv: jax.Array,
    B_wo: jax.Array,
):
    del B_x
    vmem = pltpu.VMEM
    group_bufs = [
        vmem((1, L // 2, 128), I32),
        vmem((NG // 2, L // 2, 128), I32),
        [vmem((1, 4, 64, 128), I32)] * 4,
        vmem((1, L // 2, 128), I32),
        vmem((NG // 2, 64, L), I32),
        [vmem((1, 4, 128 * (j + 1) + 24, 128), F32) for j in range(4)],
        [vmem((1, 64 * (j + 1), 512), I32) for j in range(4)],
        vmem((1, 4, 8, 128), F32),
        vmem((1, 128, L), F32),
    ]
    out = pl.pallas_call(
        _kernel,
        grid=(2 * NSEG,),
        in_specs=[pl.BlockSpec(memory_space=pl.ANY)] * 8,
        out_specs=pl.BlockSpec(memory_space=pl.ANY),
        out_shape=jax.ShapeDtypeStruct((S, D), BF16),
        scratch_shapes=[
            vmem((S, D), BF16),
            vmem((D, D), BF16),
            vmem((D, D), BF16),
            vmem((D, D), BF16),
            vmem((D, D), BF16),
            vmem((D, 3 * D), BF16),
            vmem((D, D), BF16),
            vmem((H,), BF16),
            [vmem((D // 2, D), I32)] * 4,
            [vmem((NG, NG * PST, 128), I32)] * 4,
            pltpu.SemaphoreType.DMA((3 * (len(A_SPLIT) - 1) + 6 + NR,)),
            vmem((NSEG, L, D), F32),
            vmem((L, D), F32),
            [vmem((1, 16, D), F32)] * 3,
            vmem((L, D), BF16),
            vmem((L // 2, D), I32),
            vmem((L // 2, D), I32),
            vmem((NG, 8, 128), F32),
            vmem((DH, 128), F32),
            vmem((NG, 128, 128), F32),
            vmem((NG, 1, 128), F32),
            [group_bufs] * 2,
            [vmem((1, RB, D), F32)] * NB,
            [vmem((1, RB // 2, D), I32)] * NB,
            [vmem((1, RB // 2, D), I32)] * NB,
            [vmem((1, NG, KR + RB, 128), F32)] * NB,
            [vmem((1, NG, KR, 128), F32)] * NB,
            [vmem((1, W + 1, RB, 128), F32)] * NB,
        ],
        compiler_params=pltpu.CompilerParams(
            dimension_semantics=("arbitrary",), vmem_limit_bytes=110 * 1024 * 1024),
        name="fused_layers",
    )(A_x.reshape(S, D), A_wq, A_wk, A_wv, A_wo, A_beta, B_wqkv, B_wo)
    return out.reshape(A_x.shape)
```

```python
import functools

import jax
import jax.numpy as jnp
from jax import lax
import jax.experimental.pallas as pl
import jax.experimental.pallas.tpu as pltpu

F32 = jnp.float32
BF16 = jnp.bfloat16
I32 = jnp.int32

S, D, H, DH = 2048, 1024, 32, 32
NSEG, L = 4, 512
W, DIL = 8, 2
QSCALE = DH ** -0.5 * 1.4426950408889634
NEG = -1e30

NG = D // 128
A_SPLIT = (0, 2, 8)
RB, NB = 128, 2
NR = L // (NB * RB)
HALO = 16
KR = HALO + RB
PST = 68
TICKS = 16
QK_TICKS = (3, 12, 18, 32)


def _nn(a, b):
    return jnp.dot(a, b, preferred_element_type=F32)


def _nt(a, b):
    return lax.dot_general(a, b, (((1,), (1,)), ((), ())), preferred_element_type=F32)


def _pack(x):
    return pltpu.bitcast(x.astype(BF16), I32)


def _pack_tiles(xs):
    return _tiles(_pack(jnp.concatenate(xs, axis=1)))


def _bf16(words):
    return pltpu.bitcast(words, BF16)


def _blk(i, n=128):
    return slice(i * n, (i + 1) * n)


def _ds(i, n):
    return pl.ds(i * n if isinstance(i, int) else pl.multiple_of(i * n, n), n)


def _tiles(x):
    return [x[:, _blk(t)] for t in range(x.shape[1] // 128)]


def _fold8(x, reduce=jnp.sum):
    return reduce(x.reshape(x.shape[0] // 8, 8, x.shape[1]), axis=0)


def _phi(t):
    return jnp.where(t > 0, t + 1.0, jnp.exp(t))


def _skew(xs):
    lane = lax.broadcasted_iota(I32, xs[0].shape, 1)
    for bit in (1, 2):
        swap = (lane & (bit * DH)) != 0
        xs = [lax.select(swap, xs[i ^ bit], xs[i]) for i in range(4)]
    return xs


def _skew_rows(x):
    n = x.shape[0] // 4
    return jnp.concatenate(_skew([x[_blk(i, n)] for i in range(4)]), axis=0)


def _layernorm(load, zero=None):
    x = load(0) if zero is None else jnp.concatenate([zero, load(0)], axis=1)
    m = jnp.sum(x, axis=-1, keepdims=True) * (1.0 / D)
    x = load(1) - m
    rs = lax.rsqrt(jnp.sum(x * x, axis=-1, keepdims=True) * (1.0 / D) + 1e-5)
    return _pack((load(2) - m) * rs)


class _Pacer:
    def __init__(self, z, total, now=0):
        self.z, self.total, self.now, self.due, self.waiting = z, total, now, {}, {}

    def zero(self, x):
        return (x if x.dtype == I32 else pltpu.bitcast(x, I32)) & self.z

    def deadline(self, tick, x):
        assert tick >= self.now
        if tick < self.total:
            zt = self.zero(x)
            self.due[tick] = self.due[tick] | zt if tick in self.due else zt

    def lhs(self, words, ticks=None):
        n, parts, c0 = words.shape[0] // 8, [], 0
        for c in range(0, words.shape[1], 512):
            zts = [self.due.pop(self.now + r, None) for r in range(ticks or n)]
            self.now += len(zts)
            if any(zt is not None for zt in zts):
                none = jnp.zeros((8, 128), I32)
                zts = [none if zt is None else zt for zt in zts] + [none] * (n - len(zts))
                parts += [words[:, c0:c]] if c > c0 else []
                parts.append(words[:, c:c + 128] | jnp.concatenate(zts))
                c0 = c + 128
        parts += [words[:, c0:]] if c0 < words.shape[1] else []
        return _bf16(jnp.concatenate(parts, axis=1))

    @staticmethod
    def ready(start, v):
        return start + (TICKS + v) // 2 + 7

    def at(self, points, gen):
        next(gen, None)
        for p in points:
            self.waiting.setdefault(p, []).append(gen)

    def done(self, y):
        start = self.now - TICKS
        for v in range(TICKS):
            for gen in self.waiting.pop(start + v, []):
                try:
                    gen.send((self.ready(start, v), pltpu.bitcast(self.zero(y[_blk(v, 8)]), F32)))
                except StopIteration:
                    pass

    def close(self):
        assert self.now == self.total and not self.due and not self.waiting


def _kernel(x_hbm, wq_hbm, wk_hbm, wv_hbm, wo_hbm, beta_hbm, wqkv_hbm, wob_hbm, out_hbm,
            xin, wq, wk, wv, wo, wqkv, wob, wo_head, beta, wa, wb, sems,
            xres, xcur, stage, xout, xna, oa, gate, cmask, mem_m, mem_z, group_bufs,
            xmid, xnb, ob, kq_buf, v_buf, p_buf):
    it = pl.program_id(0)
    seg = it % NSEG
    nseg = (it + 1) % NSEG
    zz = [it // (2 * NSEG << n) for n in range(3)]
    z = zz[0]
    batches = len(A_SPLIT) - 1

    def a_copies(b):
        cols = pl.ds(A_SPLIT[b] * 128, (A_SPLIT[b + 1] - A_SPLIT[b]) * 128)
        return [pltpu.make_async_copy(src.at[:, cols], dst.at[:, cols], sems.at[3 * b + i])
                for i, (src, dst) in enumerate(((wk_hbm, wk), (wq_hbm, wq), (wv_hbm, wv)))]

    def late_copies():
        pairs = ((wqkv_hbm, wqkv), (wob_hbm, wob), (wo_hbm, wo), (x_hbm.at[L:S], xin.at[L:S]))
        return [pltpu.make_async_copy(src, dst, sems.at[3 * batches + i])
                for i, (src, dst) in enumerate(pairs)]

    def out_copy(s, i):
        return pltpu.make_async_copy(xout.at[_ds(i, RB)], out_hbm.at[_ds(s * (L // RB) + i, RB)],
                                     sems.at[3 * batches + 7 + i])

    @pl.when(it == 0)
    def _start():
        beta_copy = pltpu.make_async_copy(beta_hbm, beta, sems.at[3 * batches + 4])
        x_copy = pltpu.make_async_copy(x_hbm.at[0:L], xin.at[0:L], sems.at[3 * batches + 5])
        for c in [beta_copy, x_copy] + a_copies(0):
            c.start()

        def clear(i, carry):
            xres[1:, _ds(i, 32), :] = jnp.zeros((NSEG - 1, 32, D), F32)
            return carry

        lax.fori_loop(0, L // 32, clear, 0)
        beta_copy.wait()
        g = jax.nn.sigmoid(beta[...].astype(F32).reshape(1, H))
        eye = lax.broadcasted_iota(I32, (H, H), 0) == lax.broadcasted_iota(I32, (H, H), 1)
        g = jnp.sum(jnp.where(eye, jnp.broadcast_to(g, (H, H)), 0.0), axis=1, keepdims=True)
        g = jnp.broadcast_to(g, (H, 128))
        for i in range(NG):
            gate[i] = jnp.concatenate([g[_blk(i, 4)]] * 2)
        cmask[...] = jnp.where(lax.broadcasted_iota(I32, (DH, 128), 0)
                               <= lax.broadcasted_iota(I32, (DH, 128), 1) % DH, 0.0, NEG)
        x_copy.wait()

        def first_ln(i, carry):
            x = xin[_ds(i, RB), :].astype(F32)
            xcur[_ds(i, RB), :] = x
            xna[_ds(i, RB // 2), :] = _layernorm(lambda p: xcur[_ds(i + zz[p], RB), :] if p else x)
            return carry

        lax.fori_loop(0, L // RB, first_ln, 0)

    @pl.when(seg == 0)
    def _reset():
        mem_m[...] = jnp.zeros(mem_m.shape, F32)
        mem_z[...] = jnp.zeros(mem_z.shape, F32)
        kq_buf[0][0, :, 0:HALO, :] = jnp.zeros((NG, HALO, 128), F32)
        v_buf[0][0, :, 0:HALO, :] = jnp.zeros((NG, HALO, 128), F32)

    def a_batch(b):
        first, end = A_SPLIT[b], A_SPLIT[b + 1]

        @pl.when(it == 0)
        def _weights():
            cols = slice(first * 128, end * 128)
            for n, (c, src) in enumerate(zip(a_copies(b), (wk, wq, wv))):
                c.wait()
                if n == 2:
                    head = pltpu.make_async_copy(wo_hbm.at[0:D // 2, 0:128], wo_head,
                                                 sems.at[3 * batches + 6])
                    if b == 0:
                        head.start()
                    if b == batches - 1:
                        head.wait()
                    for nxt in a_copies(b + 1) if b + 1 < batches else late_copies():
                        nxt.start()

                def to_words(i, carry, src=src, dst=wa[n]):
                    dst[_ds(i, 64), cols] = pltpu.bitcast(src[_ds(i, 128), cols], I32)
                    return carry

                lax.fori_loop(0, NG, to_words, 0)

        order = [("kq", first), ("scores", first)]
        for g in range(first + 1, end - 1):
            order += [("kq", g), ("v", g - 1), ("scores", g), ("out", g - 1), ("update", g - 1)]
        order += [("kq", end - 1), ("scores", end - 1)]
        order += [(name, g) for name in ("v", "out", "update") for g in (end - 2, end - 1)]
        order = [("filler" if name == "update" and g >= NG - 2 else name, g) for name, g in order]
        ticks = dict(kq=8 * TICKS, v=4 * TICKS, scores=sum(QK_TICKS), out=8, update=8, filler=8)
        pace = _Pacer(z, sum(ticks[name] for name, _ in order))
        lane_head = lax.broadcasted_iota(I32, (128, 128), 1) // DH
        row_head = lax.broadcasted_iota(I32, (128, 128), 0) // DH
        is_head = [lane_head[:16] == h for h in range(4)]
        none = jnp.zeros((16, 128), I32)
        swap = [(lax.broadcasted_iota(I32, (8, 128), 1) & bit) for bit in (DH, 2 * DH)]
        swap = [jnp.concatenate([bits] * 4, axis=1) != 0 for bits in swap]

        def group(g):
            ks, pks, qs, pqs, vts, ss, ps, fs, ms = group_bufs[g % 2]
            st = {}

            def proj(i, w):
                y = _nn(pace.lhs(xna[_blk(i, 64), :]), _bf16(wa[w][:, _blk(g)]))
                pace.done(y)
                return y

            def proj_kq():
                for i in range(4):
                    k = proj(i, 0)
                    pk = _phi(k)
                    ks[z, _blk(i, 64), :], pks[g // 2 + z, _blk(i, 64), :] = _pack_tiles([k, pk])
                    st["z"] = st["z"] + _fold8(pk) if i else _fold8(pk)
                for j in range(4):
                    q = proj(j, 1)
                    q, pq = _pack_tiles([q * QSCALE, _phi(q)])
                    for i in range(4):
                        qi = q[_blk(i, 16)]
                        qs[j][z, i] = jnp.concatenate([lax.select(is_head[c ^ i], qi, none) for c in range(4)])
                    pqs[z, _blk(j, 64), :] = _skew_rows(pq)

            def proj_v():
                for i in range(4):
                    vts[g // 2 + z, :, _blk(i)] = vt = pltpu.bitcast(proj(i, 2).astype(BF16).T, I32)
                    pace.deadline(pace.now + 20, vt[56:])

            def softmax(plan):
                zt = pltpu.bitcast(pace.zero(st["max", 1]), F32)
                for j in range(4):
                    sums = []
                    for r in range(0, (j + 1) * 128, 16):
                        tick, wait = next(plan)
                        zt = (yield)[1] if wait else zt
                        done = max(r // DH - 4 * j, 0)
                        if r == 0:
                            m = ss[j][0, 0:8, :]
                        if done > len(sums):
                            sums.append(l[:, :128])
                            m, l = m[:, 128:], l[:, 128:]
                        if wait or r == 0:
                            m = m + jnp.concatenate([zt] * (4 - done), axis=1)
                        e = jnp.exp2(ss[j][0, 8 + r:24 + r, done * 128:] - jnp.concatenate([m, m]))
                        l = l + _fold8(e) if r else _fold8(e)
                        e = jnp.concatenate([none[:8]] * done + [_pack(e)], axis=1)
                        e = lax.select(swap[0], jnp.concatenate([e[:, _blk(h ^ 1)] for h in range(4)], axis=1), e)
                        e = lax.select(swap[1], jnp.concatenate([e[:, 256:], e[:, :256]], axis=1), e)
                        ps[j][z, r // 2:r // 2 + 8, :] = e
                        pace.deadline(tick + 1, e[:, 384:])
                        pace.deadline(tick, functools.reduce(jnp.add, _tiles(l)))
                    total = jnp.ones((8, 128), F32)
                    for h, v in enumerate(_skew(sums + [l])):
                        total = jnp.where(lax.broadcasted_iota(I32, (8, 128), 0) == h,
                                          jnp.sum(v, axis=0, keepdims=True), total)
                    fs[z, j] = f = (1.0 - gate[g]) / total
                    pace.deadline(tick + 6, f)

            def scores():
                for j in range(4):
                    for i in (3, 2, 1, 0):
                        n = j * 128 + (i + 1) * DH
                        k = ks[0, 0:n // 2, :]
                        s = _nt(pace.lhs(k, QK_TICKS[j]) if i == 3 else _bf16(k), _bf16(qs[j][0, i]))
                        diag = s[n - DH:] + cmask[...]
                        s = jnp.concatenate([s[:n - DH], diag], axis=0) if n > DH else diag
                        ss[j][z, 8:8 + n, _blk(i)] = s
                        m = jnp.max(_fold8(s, jnp.max), axis=0, keepdims=True)
                        ss[j][z, 0:8, _blk(i)] = st["max", j] = jnp.broadcast_to(m, (8, 128))
                stop = order.index(("scores", g + 1)) + 1 if g + 1 < end else order.index(("out", g))
                slots, starts, t = [], [], pace.now
                for name, _ in order[order.index(("scores", g)) + 1:stop]:
                    if name in ("kq", "v", "scores"):
                        slots += range(t, t + ticks[name])
                    if name in ("kq", "v"):
                        starts += range(t, t + ticks[name], TICKS)
                    t += ticks[name]
                plan, points, pieces = [], [], 10 * 128 // 16
                for c in range(pieces):
                    tick = slots[c * (len(slots) - 2) // pieces]
                    early = [p + v for p in starts for v in (0, TICKS - 1) if pace.ready(p, v) + 8 <= tick]
                    plan.append((tick, bool(early) and early[-1] not in points))
                    if plan[-1][1]:
                        points.append(early[-1])
                pace.at(points, softmax(iter(plan)))

            def out():
                zrows = jnp.where(lax.broadcasted_iota(I32, (16, 128), 0) == lane_head[:16],
                                  jnp.broadcast_to(mem_z[g], (16, 128)), 0.0)
                r = _nt(jnp.concatenate([zrows, mem_m[g]], axis=0).astype(BF16), _bf16(pqs[0]))
                mem_z[g] = mem_z[g] + jnp.sum(st["z"], axis=0, keepdims=True)
                f = jnp.concatenate([gate[g]] * 4, axis=1) / (r[0:8] + 1e-6)
                for h in range(4):
                    ms[z, _blk(h, DH), :] = r[16 + h * DH:16 + (h + 1) * DH] * f[h:h + 1]
                for j in range(4):
                    heads = []
                    for h in range(4):
                        vt = vts[g // 2, _blk(h, DH // 2), 0:(j + 1) * 128]
                        o = _nn(pace.lhs(vt) if h == 3 else _bf16(vt), _bf16(ps[j][0, :, _blk(h)]))
                        heads.append(o * fs[0, j, h:h + 1, :] + ms[0, _blk(h, DH), _blk(j)])
                    o = pltpu.bitcast(jnp.concatenate(heads, axis=0).astype(BF16).T, I32)
                    oa[_blk(j, 64), _blk(g)] = o = _skew_rows(o)
                    slack = 28 if g < end - 2 else (12, 10, 9, 7)[j] if g == end - 2 else 18
                    pace.deadline(pace.now + slack, _fold8(pltpu.bitcast(o, F32)))

            def update():
                lag = (g >= NG - 2 - 2 * seg).astype(I32)
                new = _nn(pace.lhs(vts[g // 2 + lag]), _bf16(pks[g // 2 + lag]))
                mem_m[g + 2 * lag] = new = mem_m[g + 2 * lag] + jnp.where(lane_head == row_head, new, 0.0)
                pace.deadline(pace.now + 28, _fold8(new))

            def filler():
                i = (g - NG + NR) * NB
                xcur[_blk(i, RB), _blk(0)] += _nn(pace.lhs(oa[_blk(i, RB // 2), 0:D // 2]),
                                                  wo_head[...])

            return dict(kq=proj_kq, v=proj_v, scores=scores, out=out, update=update, filler=filler)

        groups = {g: group(g) for g in range(first, end)}
        for name, g in order:
            groups[g][name]()
        pace.close()

    for b in range(batches):
        a_batch(b)

    @pl.when(it == 0)
    def _reorder_b_weights():
        def move(words, dst, i, pair):
            even, odd = words[:16], words[16:]
            both = ((even & 0xFFFF) | (odd << 16), lax.shift_right_logical(even, 16) | (odd & -0x10000))
            for a in range(2):
                for c in range(2):
                    dst[i, pl.ds(32 * a + 16 * c + pair, NG, stride=PST), :] = both[c][_blk(a, 8)]

        for c in late_copies():
            c.wait()
        row = lax.broadcasted_iota(I32, (128, 128), 0)
        col = (row // 64 * 2 + row % 2) * DH + (row // 32 % 2 * 8 + row // 2 % 8) * 2 + row // 16 % 2
        mover = jnp.where(lax.broadcasted_iota(I32, (128, 128), 1) == col, 1.0, 0.0).astype(BF16)
        for i in range(NG):
            words = pltpu.bitcast(wqkv[_blk(i), 0:2 * D].T, I32)
            for pair in range(H // 2):
                for part in range(2):
                    move(words[_blk(part * (H // 2) + pair, 32)], wb[part], i, pair)
                zt = jnp.concatenate([words[_blk(8 * pair, 8)] & z] * 4)
                move(pltpu.bitcast(wob[_blk(pair, 64), _blk(i)], I32) | zt, wb[3], i, pair)
                rows, cols = 4 * i + pair // 4, _blk(pair % 4, 256)
                wa[3][_blk(rows, 16), cols] = (pltpu.bitcast(wo[_blk(rows, 32), cols], I32)
                                               | jnp.concatenate([zt[:16]] * 2, axis=1))
        for c in range(NG):
            for i0 in range(0, NG, 4):
                words = _pack(_nt(mover, wqkv[i0 * 128:(i0 + 4) * 128, _blk(2 * NG + c)]))
                for i, tile in enumerate(_tiles(words)):
                    for n in range(8):
                        wb[2][i0 + i, pl.ds(n % 4 * 16 + 2 * c + n // 4, NG, stride=PST), :] = tile[_blk(n, 8)]

    def row_trip(tr, carry):
        @pl.when(it > NSEG)
        def _sent():
            for i in range(NB):
                out_copy(jnp.maximum(seg - 1, 0), tr * NB + i).wait()

        pace = _Pacer(z, 5 * NB * NG * TICKS, TICKS // 2)

        def a_out(i, t):
            k0 = 0 if i or t else D // 2
            y = _nn(pace.lhs(oa[_ds(tr * NB + i, RB // 2), k0:]), _bf16(wa[3][k0 // 2:, _blk(t)]))
            xmid[i][z, :, _blk(t)] = xcur[_ds(tr * NB + i, RB), _blk(t)] + y
            return y

        def b_proj(i, part, t):
            y = _nt(pace.lhs(xnb[i][0]), _bf16(jnp.concatenate(
                [wb[part][k, pl.ds(t * PST, 64), :] for k in range(NG)], axis=1)))
            if part == 0:
                kq_buf[i][z, t, KR:KR + RB, :] = y * QSCALE
            else:
                buf = (kq_buf, v_buf)[part - 1]
                buf[i][z, t, HALO:KR, :] = y
                if i + 1 < NB:
                    buf[i + 1][z, t, 0:HALO, :] = y[RB - HALO:]
            return y

        def b_out(i, t):
            x = xmid[i][0, :, _blk(t)] + _nn(pace.lhs(ob[i][0]), _bf16(jnp.concatenate(
                [wb[3][t, pl.ds(k * PST, 64), :] for k in range(NG)], axis=0)))
            xres[seg, _ds(tr * NB + i, RB), _blk(t)] = x
            xout[_ds(tr * NB + i, RB), _blk(t)] = x.astype(BF16)
            if t == NG - 1:
                pl.when(it >= NSEG)(lambda: out_copy(seg, tr * NB + i).start())
            return x

        def mid_ln(i):
            for r in range(RB // 16):
                now, zt = yield
                y = _layernorm(lambda p: xmid[i][zz[p] if p else 0, _blk(r, 16), :], jnp.concatenate([zt, zt]))
                xnb[i][z, _blk(r, 8), :] = y
                pace.deadline(now + 29, y[:, D - 128:])

        def next_ln():
            n = NB * RB // 16
            for r in range(n):
                now, zt = yield
                rows = _ds(tr * n + r, 16)

                def load(p):
                    if p:
                        return stage[r % 3][zz[p]]
                    x = xin[_ds(nseg * (L // 16) + tr * n + r, 16), :].astype(F32)
                    x = jnp.where(it < NSEG - 1, x, xres[nseg, rows, :])
                    stage[r % 3][z] = x
                    xcur[rows, :] = x
                    return x

                y = _layernorm(load, jnp.concatenate([zt, zt]))
                xna[_ds(tr * n + r, 8), :] = y
                pace.deadline(now + 29, y[:, D - 128:])

        def b_softmax(i):
            for r in range(0, RB, 8):
                logits = []
                for w in range(W):
                    if w % 2 == 0:
                        now, zt = yield
                    if w == 0:
                        q = kq_buf[i][0, :, KR + r:KR + r + 8, :]
                    a = q * kq_buf[i][0, :, pl.ds(r + HALO - DIL * w, 8), :]
                    a = jnp.sum(jnp.concatenate([zt[None], a]), axis=0)
                    a = a + pltpu.roll(a, 64, 1)
                    a = a + pltpu.roll(a, 32, 1)
                    if i * RB + r < DIL * w:
                        pos = seg * L + tr * (NB * RB) + r + lax.broadcasted_iota(I32, (8, 128), 0)
                        a = jnp.where(pos >= DIL * w, a, NEG)
                    logits.append(a)
                m = functools.reduce(jnp.maximum, logits)
                es = [jnp.exp2(a - m) for a in logits]
                es.append(functools.reduce(jnp.add, es))
                for w, e in enumerate(es):
                    p_buf[i][z, w, r:r + 8, :] = e
                pace.deadline(now + 28, es[W])

        def b_mix(i):
            now, _ = yield
            for r in range(RB // 16):
                es = [p_buf[i][0, w, _blk(r, 16), :] for w in range(W)]
                inv = 1.0 / p_buf[i][0, W, _blk(r, 16), :]
                o = None
                for c in range(W // 2):
                    v = v_buf[i][0, :, pl.ds(r * 16 + HALO - DIL * c - 8, 24), :]
                    for w, vw in ((c, v[:, 8:]), (c + W // 2, v[:, :16])):
                        o = es[w] * vw if o is None else o + es[w] * vw
                o = o * inv
                for t in range(NG):
                    ob[i][z, _blk(r, 8), _blk(t)] = words = _pack(o[t])
                    pace.deadline(now + 8 + (r * NG + t) * 7 // 4, words)

        def carry_halo():
            for buf in (kq_buf, v_buf):
                _, zt = yield
                buf[0][z, :, 0:HALO, :] = buf[NB - 1][0, :, RB:KR, :] + jnp.concatenate([zt, zt])

        span = NG * TICKS
        pace.at([(5 * NB - 1) * span + n * TICKS for n in (5, 6)], carry_halo())
        for i in range(NB):
            pace.at([(i + 1) * span - 1 + 10 * n for n in range(RB // 16)], mid_ln(i))
            pace.at([(NB + 2 * i + 2) * span + (3 - i) * n for n in range(RB // 8 * W // 2)], b_softmax(i))
            pace.at([(3 * NB + i + 1) * span - 1], b_mix(i))
        pace.at([NB * span + 88 + 10 * n for n in range(NB * RB // 16)], next_ln())
        steps = [functools.partial(a_out, i) for i in range(NB)]
        steps += [functools.partial(b_proj, i, part) for i in range(NB) for part in range(2)]
        steps += [functools.partial(b_proj, i, 2) for i in range(NB)]
        steps += [functools.partial(b_out, i) for i in range(NB)]
        for step in steps:
            for t in range(NG):
                pace.done(step(t))
        pace.close()
        return carry

    lax.fori_loop(0, NR, row_trip, 0)

    @pl.when(it == 2 * NSEG - 1)
    def _finish():
        for i in range(L // RB):
            out_copy(seg, i).wait()


@jax.jit
def pallas_interleave_layers__memory_aug_infini_attn__sliding_local_dilated__prompt_kernel(
    A_x: jax.Array,
    A_wq: jax.Array,
    A_wk: jax.Array,
    A_wv: jax.Array,
    A_wo: jax.Array,
    A_beta: jax.Array,
    B_x: jax.Array,
    B_wqkv: jax.Array,
    B_wo: jax.Array,
):
    del B_x
    vmem = pltpu.VMEM
    group_bufs = [
        vmem((1, L // 2, 128), I32),
        vmem((NG // 2, L // 2, 128), I32),
        [vmem((1, 4, 64, 128), I32)] * 4,
        vmem((1, L // 2, 128), I32),
        vmem((NG // 2, 64, L), I32),
        [vmem((1, 128 * (j + 1) + 8, 512), F32) for j in range(4)],
        [vmem((1, 64 * (j + 1), 512), I32) for j in range(4)],
        vmem((1, 4, 8, 128), F32),
        vmem((1, 128, L), F32),
    ]
    out = pl.pallas_call(
        _kernel,
        grid=(2 * NSEG,),
        in_specs=[pl.BlockSpec(memory_space=pl.ANY)] * 8,
        out_specs=pl.BlockSpec(memory_space=pl.ANY),
        out_shape=jax.ShapeDtypeStruct((S, D), BF16),
        scratch_shapes=[
            vmem((S, D), BF16),
            vmem((D, D), BF16),
            vmem((D, D), BF16),
            vmem((D, D), BF16),
            vmem((D, D), BF16),
            vmem((D, 3 * D), BF16),
            vmem((D, D), BF16),
            vmem((D // 2, 128), BF16),
            vmem((H,), BF16),
            [vmem((D // 2, D), I32)] * 4,
            [vmem((NG, NG * PST + 64, 128), I32)] * 4,
            pltpu.SemaphoreType.DMA((3 * (len(A_SPLIT) - 1) + 7 + L // RB,)),
            vmem((NSEG, L, D), F32),
            vmem((L, D), F32),
            [vmem((1, 16, D), F32)] * 3,
            vmem((L, D), BF16),
            vmem((L // 2, D), I32),
            vmem((L // 2, D), I32),
            vmem((NG, 8, 128), F32),
            vmem((DH, 128), F32),
            vmem((NG, 128, 128), F32),
            vmem((NG, 1, 128), F32),
            [group_bufs] * 2,
            [vmem((1, RB, D), F32)] * NB,
            [vmem((1, RB // 2, D), I32)] * NB,
            [vmem((1, RB // 2, D), I32)] * NB,
            [vmem((1, NG, KR + RB, 128), F32)] * NB,
            [vmem((1, NG, KR, 128), F32)] * NB,
            [vmem((1, W + 1, RB, 128), F32)] * NB,
        ],
        compiler_params=pltpu.CompilerParams(
            dimension_semantics=("arbitrary",), vmem_limit_bytes=110 * 1024 * 1024),
        name="fused_layers",
    )(A_x.reshape(S, D), A_wq, A_wk, A_wv, A_wo, A_beta, B_wqkv, B_wo)
    return out.reshape(A_x.shape)
```
